```python
import os as _os
_os.environ.setdefault("JAX_PLATFORMS", "cpu")
import jax
import jax.numpy as jnp

def _softmax(x, axis=-1):
    return jax.nn.softmax(x, axis=axis)
def _gelu(x):
    return jax.nn.gelu(x, approximate=True)
def _silu(x):
    return jax.nn.silu(x)
def _sigmoid(x):
    return jax.nn.sigmoid(x)
def _layernorm(x, axis=-1, eps=1e-5):
    m = jnp.mean(x, axis=axis, keepdims=True)
    v = jnp.var(x, axis=axis, keepdims=True)
    return (x - m) / jnp.sqrt(v + eps)
def _scatter_add(tgt, idx, src, axis=0):
    return tgt.at[idx].add(src)
def _segment_sum(src, seg, n):
    return jax.ops.segment_sum(src, seg, n)
class _Rng:
    def __init__(self, key):
        self._k = key
    def _next(self):
        self._k, sub = jax.random.split(self._k)
        return sub
    def normal(self, shape):
        return jax.random.normal(self._next(), shape, dtype=jnp.bfloat16)
    def randint(self, lo, hi, shape):
        return jax.random.randint(self._next(), shape, lo, hi, dtype=jnp.int32)
    def uniform(self, shape, lo=0.0, hi=1.0):
        return jax.random.uniform(self._next(), shape, jnp.bfloat16, lo, hi)
    def permutation(self, n):
        return jax.random.permutation(self._next(), n)


kernel_name = 'concat_heads__spectral_gfnet__mha_block__prompt'

def setup_inputs():
    _rng = _Rng(jax.random.key(int.from_bytes(__import__("os").urandom(4), "little")))
    _w = (lambda a: (lambda t: t.astype(jnp.bfloat16) if jnp.issubdtype(t.dtype, jnp.floating) else t)(jnp.asarray(a)))
    def _A_setup():
        B, S, D = 1, 2048, 576
        Df = D // 2 + 1
        return {
            "x": _w((lambda *s: _rng.normal(s) * 0.05)(B, S, D)),
            "w_r": _w((lambda *s: _rng.normal(s) * 0.05)(S, Df) * 0.02),
            "w_i": _w((lambda *s: _rng.normal(s) * 0.05)(S, Df) * 0.02),
        }
    _A_in = _A_setup()

    def _B_setup():
        B, S, D, H = 1, 2048, 576, 32
        return {
            "x": _w((lambda *s: _rng.normal(s) * 0.1)(B, S, D)),
            "wqkv": _w((lambda *s: _rng.normal(s) * 0.1)(D, 3 * D)),
            "wo": _w((lambda *s: _rng.normal(s) * 0.05)(D, D)),
        }
    _B_in = _B_setup()

    return {
        "A_x": _A_in["x"],
        "A_w_r": _A_in["w_r"],
        "A_w_i": _A_in["w_i"],
        "B_x": _B_in["x"],
        "B_wqkv": _B_in["wqkv"],
        "B_wo": _B_in["wo"],
    }

def reference(A_x, A_w_r, A_w_i, B_x, B_wqkv, B_wo):
    def _A_ref(x, w_r, w_i):
        B, S, D = x.shape
        X = (lambda x, axes=(-2,-1): jnp.fft.rfft2(x.astype(jnp.float32), axes=axes))(x, axes=(-2, -1))
        W = w_r + 1j * w_i
        X = X * W
        y = (lambda x, s, axes=(-2,-1): jnp.fft.irfft2(x, s=s, axes=axes).astype(jnp.bfloat16))(X, (S, D), axes=(-2, -1))
        return y

    def _B_ref(x, wqkv, wo):
        B, S, D = x.shape
        H = 32
        Dh = D // H
        qkv = (lambda x, *d: x.transpose(*d))((x @ wqkv).reshape(B, S, 3, H, Dh), 2, 0, 3, 1, 4)
        q, k, v = qkv[0], qkv[1], qkv[2]
        scores = jnp.einsum("bhqd,bhkd->bhqk", q, k) * (Dh ** -0.5)
        p = _softmax(scores, axis=-1)
        o = jnp.einsum("bhqk,bhkd->bhqd", p, v)
        return (lambda x, *d: x.transpose(*d))(o, 0, 2, 1, 3).reshape(B, S, D) @ wo

    a = _A_ref(A_x, A_w_r, A_w_i)
    b = _B_ref(B_x, B_wqkv, B_wo)
    return jnp.concatenate([a, b], axis=-1)
```

```python
import math

import numpy as np
import jax
import jax.numpy as jnp
import jax.experimental.pallas as pl
import jax.experimental.pallas.tpu as pltpu

S = 2048
D = 576
H = 32
DH = D // H
DF = D // 2 + 1
LW = 640
TQ = 512
TC = 128
RC = 256
NQ = S // TQ
NC = S // TC
HPT = 7

_F32 = jnp.float32
_BF16 = jnp.bfloat16


def _dft_tables():
    d = np.arange(D)
    fd = np.zeros((D, LW), np.float64)
    fdi = np.zeros((LW, LW), np.float64)
    for k in range(DF):
        lr = k if k < 256 else 256 + (k - 256)
        li = 384 + k if k < 256 else 320 + (k - 256)
        ang = 2.0 * np.pi * ((d * k) % D) / D
        fd[:, lr] = np.cos(ang)
        fd[:, li] = -np.sin(ang)
        c = 1.0 if k in (0, D // 2) else 2.0
        fdi[lr, :D] = c * np.cos(ang) / (S * D)
        if k not in (0, D // 2):
            fdi[li, :D] = -c * np.sin(ang) / (S * D)
    n2 = np.arange(128)
    k2 = np.arange(128)
    g = np.zeros((16, 256, 128), np.float64)
    gh = np.zeros((16, 256, 128), np.float64)
    for k1 in range(16):
        ang = -2.0 * np.pi * (np.outer(k1 + 16 * k2, n2) % S) / S
        g[k1, :128] = np.cos(ang)
        g[k1, 128:] = np.sin(ang)
        gh[k1, :128] = np.cos(ang).T
        gh[k1, 128:] = np.sin(ang).T
    return fd, fdi, g, gh


_FD, _FDI, _G, _GH = _dft_tables()


def _cmul_w16(z, e, sign):
    re, im = z
    e = e % 16
    if e == 0:
        return z
    c = math.cos(2.0 * math.pi * e / 16.0)
    s = sign * math.sin(2.0 * math.pi * e / 16.0)
    if e == 4:
        return (-im, re) if sign > 0 else (im, -re)
    if e % 4 == 2:
        r = math.sqrt(0.5)
        a = re * r
        b = im * r
        cr = 1.0 if c > 0 else -1.0
        sr = 1.0 if s > 0 else -1.0
        nre = (a if cr > 0 else -a) - (b if sr > 0 else -b)
        nim = (a if sr > 0 else -a) + (b if cr > 0 else -b)
        return nre, nim
    return re * c - im * s, re * s + im * c


def _dft4(x0, x1, x2, x3, sign):
    e = (x0[0] + x2[0], x0[1] + x2[1])
    f = (x0[0] - x2[0], x0[1] - x2[1])
    g = (x1[0] + x3[0], x1[1] + x3[1])
    h = (x1[0] - x3[0], x1[1] - x3[1])
    y0 = (e[0] + g[0], e[1] + g[1])
    y2 = (e[0] - g[0], e[1] - g[1])
    if sign > 0:
        y1 = (f[0] - h[1], f[1] + h[0])
        y3 = (f[0] + h[1], f[1] - h[0])
    else:
        y1 = (f[0] + h[1], f[1] - h[0])
        y3 = (f[0] - h[1], f[1] + h[0])
    return y0, y1, y2, y3


def _dft16(xs, sign):
    t = [_dft4(xs[b], xs[4 + b], xs[8 + b], xs[12 + b], sign) for b in range(4)]
    t = [[_cmul_w16(t[b][c], b * c, sign) for c in range(4)] for b in range(4)]
    out = [None] * 16
    for c in range(4):
        ys = _dft4(t[0][c], t[1][c], t[2][c], t[3][c], sign)
        for dd in range(4):
            out[c + 4 * dd] = ys[dd]
    return out


def _kernel(xat_hbm, wrt_hbm, wit_hbm, xbt_hbm, wqkv_hbm, wo_hbm,
            fd_hbm, fdi_hbm, g_hbm, gh_hbm,
            out_hbm,
            xat_ref, wrt_ref, wit_ref, xbt_ref, wqkv_ref, wo_ref,
            fd_ref, fdi_ref, g_ref, gh_ref,
            out_scr, in_sems, out_sems,
            k_scr, qt_scr, vt_scr, ot_scr, sbuf, mbuf,
            wk_scr, wqt_scr, wvt_scr, wo_scr,
            y_scr, w_scr, mid_scr):
    srcs = (wqkv_hbm, xbt_hbm, xat_hbm, fd_hbm, wrt_hbm, wit_hbm, wo_hbm, g_hbm, gh_hbm, fdi_hbm)
    dsts = (wqkv_ref, xbt_ref, xat_ref, fd_ref, wrt_ref, wit_ref, wo_ref, g_ref, gh_ref, fdi_ref)
    copies = [pltpu.make_async_copy(s, d, in_sems.at[i])
              for i, (s, d) in enumerate(zip(srcs, dsts))]
    copies[0].start()
    copies[1].start()

    copies[0].wait()
    for t in range(5):
        wk_scr[:, 128 * t:128 * (t + 1)] = wqkv_ref[:, D + 126 * t:D + 126 * t + 128]
        wqt_scr[128 * t:128 * (t + 1), :] = wqkv_ref[:, 126 * t:126 * t + 128].T
    wvt_scr[...] = wqkv_ref[:, 2 * D:3 * D].T
    mid_scr[pl.ds((NQ - 1) * TQ, TQ), :] = jnp.zeros((TQ, 128), _F32)

    qscale = (DH ** -0.5) * math.log2(math.e)
    copies[1].wait()
    for cp in copies[2:]:
        cp.start()

    def proj_body(i, carry):
        r0 = pl.multiple_of(i * RC, RC)
        xt = xbt_ref[:, pl.ds(r0, RC)]
        qt = jnp.dot(wqt_scr[...], xt, preferred_element_type=_F32)
        qt_scr[:, pl.ds(r0, RC)] = (qt * qscale).astype(_BF16)
        vt = jnp.dot(wvt_scr[...], xt, preferred_element_type=_F32)
        vt_scr[:, pl.ds(r0, RC)] = vt.astype(_BF16).astype(_F32)
        k_scr[pl.ds(r0, RC), :] = jnp.dot(
            xt.T, wk_scr[...], preferred_element_type=_F32).astype(_BF16)
        return carry

    jax.lax.fori_loop(0, S // RC, proj_body, 0)

    for i in range(2, 6):
        copies[i].wait()

    def apre_body(i, carry):
        r0 = pl.multiple_of(i * RC, RC)
        y_scr[pl.ds(r0, RC), :] = jnp.dot(
            xat_ref[:, pl.ds(r0, RC)].T, fd_ref[...], preferred_element_type=_F32)
        wr = wrt_ref[:, pl.ds(r0, RC)].T.astype(_F32)
        wi = wit_ref[:, pl.ds(r0, RC)].T.astype(_F32)
        w_scr[0, pl.ds(r0, RC), :] = wr[:, 0:128]
        w_scr[1, pl.ds(r0, RC), :] = wr[:, 128:256]
        w_scr[3, pl.ds(r0, RC), :] = wi[:, 0:128]
        w_scr[4, pl.ds(r0, RC), :] = wi[:, 128:256]
        z = jnp.zeros((RC, 128), _F32)
        w_scr[2, pl.ds(r0, RC), :] = z
        w_scr[5, pl.ds(r0, RC), :] = z
        w_scr[2, pl.ds(r0, RC), 0:33] = wr[:, 256:289]
        w_scr[2, pl.ds(r0, RC), 64:97] = wr[:, 256:289]
        w_scr[5, pl.ds(r0, RC), 0:33] = -wi[:, 256:289]
        w_scr[5, pl.ds(r0, RC), 64:97] = wi[:, 256:289]
        return carry

    jax.lax.fori_loop(0, S // RC, apre_body, 0)

    for i in range(6, 10):
        copies[i].wait()
    wo_scr[:, 0:64] = jnp.zeros((D, 64), _BF16)
    wo_scr[:, 64:128] = wo_ref[:, 0:64]
    for j in range(1, 5):
        wo_scr[:, 128 * j:128 * (j + 1)] = wo_ref[:, 128 * j - 64:128 * j + 64]

    lane8 = jax.lax.broadcasted_iota(jnp.int32, (8, 128), 1)
    lane128 = jax.lax.broadcasted_iota(jnp.int32, (128, 128), 1)
    sgn_lo_neg = jnp.where(lane128 < 64, -1.0, 1.0).astype(_F32)

    def bfly_slice(i, sign):
        r0 = pl.multiple_of(i * 8, 8)
        for (tr, ti) in ((0, 3), (1, 4)):
            xs = [(y_scr[pl.ds(128 * n + r0, 8), 128 * tr:128 * (tr + 1)],
                   y_scr[pl.ds(128 * n + r0, 8), 128 * ti:128 * (ti + 1)])
                  for n in range(16)]
            ys = _dft16(xs, sign)
            for n in range(16):
                y_scr[pl.ds(128 * n + r0, 8), 128 * tr:128 * (tr + 1)] = ys[n][0]
                y_scr[pl.ds(128 * n + r0, 8), 128 * ti:128 * (ti + 1)] = ys[n][1]
        ms = [y_scr[pl.ds(128 * n + r0, 8), 256:384] for n in range(16)]
        xs = [(m, pltpu.roll(m, 64, 1)) for m in ms]
        ys = _dft16(xs, sign)
        for n in range(16):
            y_scr[pl.ds(128 * n + r0, 8), 256:384] = jnp.where(
                lane8 < 64, ys[n][0], pltpu.roll(ys[n][1], 64, 1))

    def smid_slice(k1):
        r0 = pl.multiple_of(k1 * 128, 128)
        a = y_scr[pl.ds(r0, 128), :].astype(_BF16)
        p = jnp.dot(g_ref[k1], a, preferred_element_type=_F32)
        p1 = p[:128]
        p2 = p[128:]
        xr0 = p1[:, 0:128] - p2[:, 384:512]
        xi0 = p1[:, 384:512] + p2[:, 0:128]
        xr1 = p1[:, 128:256] - p2[:, 512:640]
        xi1 = p1[:, 512:640] + p2[:, 128:256]
        xm = p1[:, 256:384] + sgn_lo_neg * pltpu.roll(p2[:, 256:384], 64, 1)
        w = [w_scr[t, pl.ds(k1, 128, stride=16), :] for t in range(6)]
        zr0 = xr0 * w[0] - xi0 * w[3]
        zi0 = xr0 * w[3] + xi0 * w[0]
        zr1 = xr1 * w[1] - xi1 * w[4]
        zi1 = xr1 * w[4] + xi1 * w[1]
        zm = xm * w[2] + pltpu.roll(xm, 64, 1) * w[5]
        z = jnp.concatenate([zr0, zr1, zm, zi0, zi1], axis=1).astype(_BF16)
        q = jnp.dot(gh_ref[k1], z, preferred_element_type=_F32)
        q1 = q[:128]
        q2 = q[128:]
        y_scr[pl.ds(r0, 128), 0:128] = q1[:, 0:128] + q2[:, 384:512]
        y_scr[pl.ds(r0, 128), 384:512] = q1[:, 384:512] - q2[:, 0:128]
        y_scr[pl.ds(r0, 128), 128:256] = q1[:, 128:256] + q2[:, 512:640]
        y_scr[pl.ds(r0, 128), 512:640] = q1[:, 512:640] - q2[:, 128:256]
        y_scr[pl.ds(r0, 128), 256:384] = (
            q1[:, 256:384] - sgn_lo_neg * pltpu.roll(q2[:, 256:384], 64, 1))

    def dinv_slice(i):
        r0 = pl.multiple_of(i * 128, 128)
        y = jnp.dot(y_scr[pl.ds(r0, 128), :].astype(_BF16), fdi_ref[...],
                    preferred_element_type=_F32)
        out_scr[pl.ds(r0, 128), 0:512] = y[:, 0:512].astype(_BF16)
        t = y[:, 512:640] + mid_scr[pl.ds(r0, 128), :]
        mid_scr[pl.ds(r0, 128), :] = t
        out_scr[pl.ds(r0, 128), 512:640] = t.astype(_BF16)

    a_slices = (lambda i: bfly_slice(i, -1), smid_slice,
                lambda i: bfly_slice(i, 1), dinv_slice)

    U = NQ * H
    rows128 = jax.lax.broadcasted_iota(jnp.int32, (128, TQ), 0)
    rows32q = jax.lax.broadcasted_iota(jnp.int32, (24, TQ), 0)
    rows32c = jax.lax.broadcasted_iota(jnp.int32, (24, TC), 0)

    def qk_w(u):
        u = jnp.minimum(u, U - 1)
        qb = u // H
        h = u % H
        t = h // HPT
        j = h % HPT
        q0 = pl.multiple_of(qb * TQ, TQ)
        t0 = pl.multiple_of(t * 128, 128)
        qt = qt_scr[pl.ds(t0, 128), pl.ds(q0, TQ)]
        mask = (rows128 >= j * DH) & (rows128 < (j + 1) * DH)
        return jnp.where(mask, qt, jnp.zeros_like(qt)), t0

    def qk_c(qm, t0, c, slot, m):
        kt = k_scr[c * TC:(c + 1) * TC, pl.ds(t0, 128)]
        s = jnp.dot(kt, qm, preferred_element_type=_F32)
        sbuf[slot, c * TC:(c + 1) * TC, :] = s
        mc = jnp.max(s.reshape(TC // 8, 8, TQ), axis=0)
        return mc if m is None else jnp.maximum(m, mc)

    def step(qb, h, par):
        u = qb * H + h
        st = pl.multiple_of(((h * DH) // 8) * 8, 8)
        off = h * DH - st
        r1 = (off + DH) % 24
        qm, t0 = qk_w(u + 1)
        m = None
        o = None
        for c in range(NC):
            m = qk_c(qm, t0, c, 1 - par, m)
            p = jnp.exp2(sbuf[par, c * TC:(c + 1) * TC, :] - mbuf[par]).astype(_BF16)
            vw = vt_scr[pl.ds(st, 24), c * TC:(c + 1) * TC]
            vw = jnp.where(rows32c == r1, jnp.ones_like(vw), vw)
            oc = jnp.dot(vw, p, preferred_element_type=_F32)
            o = oc if o is None else o + oc
        mbuf[1 - par] = jnp.max(m, axis=0, keepdims=True)
        l = jnp.sum(jnp.where(rows32q == r1, o, 0.0), axis=0, keepdims=True)
        o = o * (1.0 / l)
        omask = (rows32q >= off) & (rows32q < off + DH)
        pltpu.store(ot_scr.at[pl.ds(st, 24), qb * TQ:(qb + 1) * TQ], o, mask=omask)

    qm0, t00 = qk_w(0)
    m0 = None
    for c in range(NC):
        m0 = qk_c(qm0, t00, c, 0, m0)
    mbuf[0] = jnp.max(m0, axis=0, keepdims=True)

    tn = (((0,), (0,)), ((), ()))
    out_copies = []
    for qb in range(NQ):
        def heads_body(i, c2, qb=qb):
            step(qb, 2 * i, 0)
            a_slices[qb](i)
            step(qb, 2 * i + 1, 1)
            return c2

        jax.lax.fori_loop(0, H // 2, heads_body, 0)
        q0 = qb * TQ
        ob = ot_scr[:, q0:q0 + TQ].astype(_BF16)
        b = jax.lax.dot_general(ob, wo_scr[...], tn, preferred_element_type=_F32)
        out_scr[q0:q0 + TQ, 640:1152] = b[:, 128:640].astype(_BF16)
        if qb < NQ - 1:
            mid_scr[q0:q0 + TQ, :] = b[:, 0:128]
            cp = pltpu.make_async_copy(out_scr.at[q0:q0 + TQ, 640:1152],
                                       out_hbm.at[q0:q0 + TQ, 640:1152], out_sems.at[qb])
            cp.start()
            out_copies.append(cp)
        else:
            cp = pltpu.make_async_copy(out_scr.at[0:q0, 0:640],
                                       out_hbm.at[0:q0, 0:640], out_sems.at[NQ])
            cp.start()
            out_copies.append(cp)
            out_scr[q0:q0 + TQ, 512:640] = (
                b[:, 0:128] + mid_scr[q0:q0 + TQ, :]).astype(_BF16)
            cp = pltpu.make_async_copy(out_scr.at[q0:q0 + TQ, :],
                                       out_hbm.at[q0:q0 + TQ, :], out_sems.at[qb])
            cp.start()
            out_copies.append(cp)
    for cp in out_copies:
        cp.wait()


@jax.jit
def pallas_concat_heads__spectral_gfnet__mha_block__prompt_kernel(
    A_x: jax.Array,
    A_w_r: jax.Array,
    A_w_i: jax.Array,
    B_x: jax.Array,
    B_wqkv: jax.Array,
    B_wo: jax.Array,
):
    xat = A_x.reshape(S, D).T
    xbt = B_x.reshape(S, D).T
    wrt = A_w_r.T
    wit = A_w_i.T
    fd = jnp.asarray(_FD, dtype=_BF16)
    fdi = jnp.asarray(_FDI, dtype=_BF16)
    g = jnp.asarray(_G, dtype=_BF16)
    gh = jnp.asarray(_GH, dtype=_BF16)

    any_spec = pl.BlockSpec(memory_space=pl.ANY)
    out = pl.pallas_call(
        _kernel,
        out_shape=jax.ShapeDtypeStruct((S, 2 * D), _BF16),
        in_specs=[any_spec] * 10,
        out_specs=any_spec,
        scratch_shapes=[
            pltpu.VMEM((D, S), _BF16),
            pltpu.VMEM((DF, S), _BF16),
            pltpu.VMEM((DF, S), _BF16),
            pltpu.VMEM((D, S), _BF16),
            pltpu.VMEM((D, 3 * D), _BF16),
            pltpu.VMEM((D, D), _BF16),
            pltpu.VMEM((D, LW), _BF16),
            pltpu.VMEM((LW, LW), _BF16),
            pltpu.VMEM((16, 256, 128), _BF16),
            pltpu.VMEM((16, 256, 128), _BF16),
            pltpu.VMEM((S, 2 * D), _BF16),
            pltpu.SemaphoreType.DMA((10,)),
            pltpu.SemaphoreType.DMA((NQ + 1,)),
            pltpu.VMEM((S, LW), _BF16),
            pltpu.VMEM((LW, S), _BF16),
            pltpu.VMEM((D, S), _F32),
            pltpu.VMEM((D, S), _F32),
            pltpu.VMEM((2, S, TQ), _F32),
            pltpu.VMEM((2, 1, TQ), _F32),
            pltpu.VMEM((D, LW), _BF16),
            pltpu.VMEM((LW, D), _BF16),
            pltpu.VMEM((D, D), _BF16),
            pltpu.VMEM((D, LW), _BF16),
            pltpu.VMEM((S, LW), _F32),
            pltpu.VMEM((6, S, 128), _F32),
            pltpu.VMEM((S, 128), _F32),
        ],
        compiler_params=pltpu.CompilerParams(vmem_limit_bytes=100 * 1024 * 1024),
    )(xat, wrt, wit, xbt, B_wqkv, B_wo, fd, fdi, g, gh)
    return out.reshape(1, S, 2 * D)
```

```python
import functools
import math

import numpy as np
import jax
import jax.numpy as jnp
import jax.experimental.pallas as pl
import jax.experimental.pallas.tpu as pltpu

S = 2048
D = 576
H = 32
DH = D // H
DF = D // 2 + 1
LW = 640
TQ = 512
TC = 128
RC = 256
NQ = S // TQ
NC = S // TC
LAG = 2
QR = 592
HPT = 7
NR = 296
NG = NR // 8

_F32 = jnp.float32
_BF16 = jnp.bfloat16


def _dft_tables():
    n2 = np.arange(64)
    mf = np.zeros((5, 128, 128), np.float64)
    mi = np.zeros((5, 128, 128), np.float64)
    for k1 in range(1, 5):
        for part, base in ((0, k1), (1, 9 - k1)):
            sg = 1.0 if part == 0 else -1.0
            for j in range(32):
                k = base + 9 * j
                ang = 2.0 * np.pi * ((n2 * k) % D) / D
                c, s = np.cos(ang), np.sin(ang)
                rr = 32 * part + j
                ri = 64 + 32 * part + j
                mf[k1 - 1, rr, :64] = c
                mf[k1 - 1, rr, 64:] = sg * s
                mf[k1 - 1, ri, :64] = -s
                mf[k1 - 1, ri, 64:] = sg * c
                f = 2.0 / (S * D)
                mi[k1 - 1, :64, rr] = f * c
                mi[k1 - 1, :64, ri] = -f * s
                mi[k1 - 1, 64:, rr] = f * sg * s
                mi[k1 - 1, 64:, ri] = f * sg * c
    for j in range(33):
        k = 9 * j
        ang = 2.0 * np.pi * ((n2 * k) % D) / D
        c, s = np.cos(ang), np.sin(ang)
        mf[4, j, :64] = c
        mf[4, 40 + j, :64] = -s
        f = (1.0 if j in (0, 32) else 2.0) / (S * D)
        mi[4, :64, j] = f * c
        if j not in (0, 32):
            mi[4, :64, 40 + j] = -f * s
    m2 = np.arange(128)
    gt = np.zeros((16, 128, 256), np.float64)
    gi = np.zeros((16, 128, 256), np.float64)
    for k1 in range(16):
        ang = -2.0 * np.pi * (np.outer(k1 + 16 * m2, m2) % S) / S
        gt[k1, :, :128] = np.cos(ang).T
        gt[k1, :, 128:] = np.sin(ang).T
        gi[k1, :, :128] = np.cos(ang)
        gi[k1, :, 128:] = np.sin(ang)
    return mf, mi, gt, gi


_MF, _MI, _GT, _GI = _dft_tables()
_C9 = [[math.cos(2.0 * math.pi * j * k / 9.0) for k in range(5)] for j in range(5)]
_S9 = [[math.sin(2.0 * math.pi * j * k / 9.0) for k in range(5)] for j in range(5)]


def _cmul_w16(z, e, sign):
    re, im = z
    e = e % 16
    if e == 0:
        return z
    c = math.cos(2.0 * math.pi * e / 16.0)
    s = sign * math.sin(2.0 * math.pi * e / 16.0)
    if e == 4:
        return (-im, re) if sign > 0 else (im, -re)
    if e % 4 == 2:
        r = math.sqrt(0.5)
        a = re * r
        b = im * r
        cr = 1.0 if c > 0 else -1.0
        sr = 1.0 if s > 0 else -1.0
        nre = (a if cr > 0 else -a) - (b if sr > 0 else -b)
        nim = (a if sr > 0 else -a) + (b if cr > 0 else -b)
        return nre, nim
    return re * c - im * s, re * s + im * c


def _dft4(x0, x1, x2, x3, sign):
    e = (x0[0] + x2[0], x0[1] + x2[1])
    f = (x0[0] - x2[0], x0[1] - x2[1])
    g = (x1[0] + x3[0], x1[1] + x3[1])
    h = (x1[0] - x3[0], x1[1] - x3[1])
    y0 = (e[0] + g[0], e[1] + g[1])
    y2 = (e[0] - g[0], e[1] - g[1])
    if sign > 0:
        y1 = (f[0] - h[1], f[1] + h[0])
        y3 = (f[0] + h[1], f[1] - h[0])
    else:
        y1 = (f[0] + h[1], f[1] - h[0])
        y3 = (f[0] - h[1], f[1] + h[0])
    return y0, y1, y2, y3


def _dft16(xs, sign):
    t = [_dft4(xs[b], xs[4 + b], xs[8 + b], xs[12 + b], sign) for b in range(4)]
    t = [[_cmul_w16(t[b][c], b * c, sign) for c in range(4)] for b in range(4)]
    out = [None] * 16
    for c in range(4):
        ys = _dft4(t[0][c], t[1][c], t[2][c], t[3][c], sign)
        for dd in range(4):
            out[c + 4 * dd] = ys[dd]
    return out


def _lin(terms):
    acc = None
    for cf, arr in terms:
        if abs(cf) < 1e-12:
            continue
        if abs(cf - 1.0) < 1e-12:
            acc = arr if acc is None else acc + arr
        elif abs(cf + 1.0) < 1e-12:
            acc = -arr if acc is None else acc - arr
        else:
            t = arr * cf
            acc = t if acc is None else acc + t
    return acc


def _kernel(xat_hbm, wrt_hbm, wit_hbm, xbt_hbm, wqkv_hbm, wo_hbm,
            mf_hbm, mi_hbm, gt_hbm, gi_hbm,
            out_hbm,
            xat_ref, wrt_ref, wit_ref, xbt_ref, wqkv_ref, wo_ref,
            mf_ref, mi_ref, gt_ref, gi_ref,
            out_scr, in_sems, out_sems, a_sems, w_sems, x_sems,
            k_scr, qt_scr, vt_scr, ot_scr, sbuf, mbuf,
            wk_scr, wqt_scr, wvt_scr, wo_scr,
            y_scr, y2_scr, w_scr, wt_scr, wp_scr, qm_scr, mpart, oacc):
    srcs = (xat_hbm, mf_hbm, wrt_hbm, wit_hbm, wo_hbm, gt_hbm, gi_hbm, mi_hbm)
    dsts = (xat_ref, mf_ref, wrt_ref, wit_ref, wo_ref, gt_ref, gi_ref, mi_ref)
    copies = [pltpu.make_async_copy(s, d, in_sems.at[i])
              for i, (s, d) in enumerate(zip(srcs, dsts))]
    wcols = ((0, 640), (640, 1280), (1280, 3 * D))
    wcopies = [pltpu.make_async_copy(wqkv_hbm.at[:, a:b], wqkv_ref.at[:, a:b], w_sems.at[i])
               for i, (a, b) in enumerate(wcols)]

    def x_copy(c0, i):
        return pltpu.make_async_copy(xbt_hbm.at[:, pl.ds(c0, RC)],
                                     xbt_ref.at[:, pl.ds(c0, RC)], x_sems.at[i])

    wcopies[0].start()
    wcopies[1].start()

    wcopies[0].wait()
    wcopies[2].start()
    x_copy(0, 0).start()
    for t in range(5):
        n = 128 if t < 4 else QR - 512
        wqt_scr[128 * t:128 * t + n, :] = wqkv_ref[:, 126 * t:126 * t + 128].T[0:n]
    wcopies[1].wait()
    for i in range(1, S // RC):
        x_copy(i * RC, i).start()
    for t in range(5):
        n = 128 if t < 4 else QR - 512
        wk_scr[128 * t:128 * t + n, :] = wqkv_ref[:, D + 126 * t:D + 126 * t + 128].T[0:n]
    wcopies[2].wait()
    wvt_scr[...] = wqkv_ref[:, 2 * D:3 * D].T

    qscale = (DH ** -0.5) * math.log2(math.e)
    for cp in copies:
        cp.start()

    def proj(i):
        r0 = pl.multiple_of(i * RC, RC)
        x_copy(r0, i).wait()
        xt = xbt_ref[:, pl.ds(r0, RC)]
        kt = jnp.dot(wk_scr[...], xt, preferred_element_type=_F32).astype(_BF16)
        kt = jnp.concatenate([kt, jnp.zeros((LW - QR, RC), _BF16)], axis=0)
        k_scr[pl.ds(r0, RC), :] = kt.T
        qt = jnp.dot(wqt_scr[...], xt, preferred_element_type=_F32)
        qt_scr[0:QR, pl.ds(r0, RC)] = (qt * qscale).astype(_BF16)
        vt = jnp.dot(wvt_scr[...], xt, preferred_element_type=_F32)
        vt_scr[:, pl.ds(r0, RC)] = vt.astype(_BF16).astype(_F32)

    def dfwd_tile(l0):
        xt = xat_ref[:, pl.ds(l0, 128)].astype(_F32)
        xb = [xt[64 * n:64 * (n + 1)] for n in range(9)]
        u = [None] + [xb[j] + xb[9 - j] for j in range(1, 5)]
        v = [None] + [xb[j] - xb[9 - j] for j in range(1, 5)]
        for k in range(1, 5):
            ar = _lin([(1.0, xb[0])] + [(_C9[j][k], u[j]) for j in range(1, 5)])
            ai = _lin([(-_S9[j][k], v[j]) for j in range(1, 5)])
            a = jnp.concatenate([ar, ai], axis=0).astype(_BF16)
            o = jnp.dot(mf_ref[k - 1], a, preferred_element_type=_F32)
            y_scr[64 * (k - 1):64 * k, pl.ds(l0, 128)] = o[:64]
            y_scr[NR + 64 * (k - 1):NR + 64 * k, pl.ds(l0, 128)] = o[64:]
        a0 = (xb[0] + (u[1] + u[2]) + (u[3] + u[4])).astype(_BF16)
        o = jnp.dot(mf_ref[4, 0:80, 0:64], a0, preferred_element_type=_F32)
        y_scr[256:NR, pl.ds(l0, 128)] = o[:40]
        y_scr[NR + 256:2 * NR, pl.ds(l0, 128)] = o[40:]

    def wnat_chunk(r0):
        wr = wrt_ref[:, pl.ds(r0, 256)].T.astype(_F32)
        wi = wit_ref[:, pl.ds(r0, 256)].T.astype(_F32)
        z = jnp.zeros((256, 128), _F32)
        for p, w in ((0, wr), (1, wi)):
            w_scr[3 * p + 0, pl.ds(r0, 256), :] = w[:, 0:128]
            w_scr[3 * p + 1, pl.ds(r0, 256), :] = w[:, 128:256]
            w_scr[3 * p + 2, pl.ds(r0, 256), :] = z
            w_scr[3 * p + 2, pl.ds(r0, 256), 0:33] = w[:, 256:289]

    def proj_body1(i, carry):
        proj(i)
        return carry

    jax.lax.fori_loop(0, 4, proj_body1, 0)

    for i in range(0, 4):
        copies[i].wait()

    def proj_body2(i, carry):
        proj(4 + i)
        for j in range(4):
            dfwd_tile(pl.multiple_of(i * 512 + j * 128, 128))
        for j in range(2):
            wnat_chunk(pl.multiple_of(i * 512 + j * 256, 256))
        return carry

    jax.lax.fori_loop(0, 4, proj_body2, 0)

    for i in range(4, 8):
        copies[i].wait()
    wo_scr[...] = wo_ref[...].T

    def bfly_group(g, sign):
        r0 = pl.multiple_of(jnp.minimum(g, NG - 1) * 8, 8)
        xs = [(y_scr[pl.ds(r0, 8), 128 * n:128 * (n + 1)],
               y_scr[pl.ds(NR + r0, 8), 128 * n:128 * (n + 1)]) for n in range(16)]
        ys = _dft16(xs, sign)
        for n in range(16):
            y2_scr[pl.ds(r0, 8), 128 * n:128 * (n + 1)] = ys[n][0]
            y2_scr[pl.ds(NR + r0, 8), 128 * n:128 * (n + 1)] = ys[n][1]

    def wperm_slice(k1s):
        l0 = pl.multiple_of(k1s * 128, 128)
        for p in range(2):
            for t in range(3):
                blk = w_scr[3 * p + t, pl.ds(k1s, 128, stride=16), :]
                wt_scr[p, 128 * t:128 * (t + 1), :] = blk.T
            for k in range(1, 5):
                wp_scr[NR * p + 64 * (k - 1):NR * p + 64 * (k - 1) + 32, pl.ds(l0, 128)] = (
                    wt_scr[p, pl.ds(k, 32, stride=9), :])
                wp_scr[NR * p + 64 * (k - 1) + 32:NR * p + 64 * k, pl.ds(l0, 128)] = (
                    wt_scr[p, pl.ds(9 - k, 32, stride=9), :])
            wp_scr[NR * p + 256:NR * (p + 1), pl.ds(l0, 128)] = (
                wt_scr[p, pl.ds(0, 40, stride=9), :])

    def stage_bfly_fwd(i):
        return [(1, lambda: bfly_group(3 * i, -1)),
                (6, lambda: bfly_group(3 * i + 1, -1)),
                (11, lambda: bfly_group(3 * i + 2, -1)),
                (18, lambda: wperm_slice(i))]

    def stage_bfly_inv(i):
        return [(1, lambda: bfly_group(3 * i, 1)),
                (10, lambda: bfly_group(3 * i + 1, 1)),
                (20, lambda: bfly_group(3 * i + 2, 1))]

    def stage_smid(k1s):
        l0 = pl.multiple_of(k1s * 128, 128)
        st = {}

        def part_a():
            st["p"] = jnp.dot(y2_scr[:, pl.ds(l0, 128)], gt_ref[k1s],
                              preferred_element_type=_F32)

        def part_b():
            p = st["p"]
            xr = p[:NR, :128] - p[NR:, 128:]
            xi = p[NR:, :128] + p[:NR, 128:]
            wpr = wp_scr[0:NR, pl.ds(l0, 128)]
            wpi = wp_scr[NR:2 * NR, pl.ds(l0, 128)]
            z = jnp.concatenate([xr * wpr - xi * wpi, xr * wpi + xi * wpr], axis=0)
            st["q"] = jnp.dot(z, gi_ref[k1s], preferred_element_type=_F32)

        def part_c():
            q = st["q"]
            y_scr[0:NR, pl.ds(l0, 128)] = q[:NR, :128] + q[NR:, 128:]
            y_scr[NR:2 * NR, pl.ds(l0, 128)] = q[NR:, :128] - q[:NR, 128:]

        return [(2, part_a), (12, part_b), (22, part_c)]

    def a_copy(r0, j):
        return pltpu.make_async_copy(out_scr.at[pl.ds(r0, 128), 0:512],
                                     out_hbm.at[pl.ds(r0, 128), 0:512], a_sems.at[j])

    def stage_dinv(j):
        l0 = pl.multiple_of(j * 128, 128)
        st = {}

        def part_a():
            cs = []
            for k in range(1, 5):
                zz = jnp.concatenate(
                    [y2_scr[64 * (k - 1):64 * k, pl.ds(l0, 128)],
                     y2_scr[NR + 64 * (k - 1):NR + 64 * k, pl.ds(l0, 128)]],
                    axis=0).astype(_BF16)
                cs.append(jnp.dot(mi_ref[k - 1], zz, preferred_element_type=_F32))
            zz = jnp.concatenate(
                [y2_scr[256:NR, pl.ds(l0, 128)],
                 y2_scr[NR + 256:2 * NR, pl.ds(l0, 128)]], axis=0).astype(_BF16)
            st["c0"] = jnp.dot(mi_ref[4, 0:64, 0:80], zz, preferred_element_type=_F32)
            st["cs"] = cs

        def part_b():
            c0 = st["c0"]
            cr = [None] + [c[:64] for c in st["cs"]]
            ci = [None] + [c[64:] for c in st["cs"]]
            ys = [None] * 9
            ys[0] = c0 + (cr[1] + cr[2]) + (cr[3] + cr[4])
            for n in range(1, 5):
                e = _lin([(1.0, c0)] + [(_C9[n][k], cr[k]) for k in range(1, 5)])
                o = _lin([(_S9[n][k], ci[k]) for k in range(1, 5)])
                ys[n] = e - o
                ys[9 - n] = e + o
            yt = jnp.concatenate(ys, axis=0).astype(_BF16)
            out_scr[pl.ds(l0, 128), 0:D] = yt.T

        def part_c():
            a_copy(l0, j).start()

        return [(2, part_a), (12, part_b), (2 * NC - 1, part_c)]

    a_stages = (stage_bfly_fwd, stage_smid, stage_bfly_inv, stage_dinv)

    U = NQ * H
    rows128 = jax.lax.broadcasted_iota(jnp.int32, (128, TQ), 0)
    rows24q = jax.lax.broadcasted_iota(jnp.int32, (24, TQ), 0)
    rows24c = jax.lax.broadcasted_iota(jnp.int32, (24, TC), 0)

    def div7(h):
        return (h * 37) >> 8

    def tile_of(u):
        h = jnp.minimum(u, U - 1) & (H - 1)
        return pl.multiple_of(div7(h) * 128, 128)

    def qk_w(u):
        u = jnp.minimum(u, U - 1)
        qb = u >> 5
        h = u & (H - 1)
        j = h - div7(h) * HPT
        q0 = pl.multiple_of(qb * TQ, TQ)
        qt = qt_scr[pl.ds(tile_of(u), 128), pl.ds(q0, TQ)]
        mask = (rows128 >= j * DH) & (rows128 < (j + 1) * DH)
        return jnp.where(mask, qt, jnp.zeros_like(qt))

    def qk_c(qm, t0, c, slot, m):
        kt = k_scr[c * TC:(c + 1) * TC, pl.ds(t0, 128)]
        s = jnp.dot(kt, qm, preferred_element_type=_F32)
        sbuf[slot, c * TC:(c + 1) * TC, :] = s
        mc = jnp.max(s.reshape(TC // 8, 8, TQ), axis=0)
        return mc if m is None else jnp.maximum(m, mc)

    def head_rows(h):
        st = pl.multiple_of(((h * DH) >> 3) * 8, 8)
        off = h * DH - st
        return st, off, jnp.where(off == 6, 0, off + DH)

    def pv_c(st, r1, c, slot, mrow, o):
        p = jnp.exp2(sbuf[slot, c * TC:(c + 1) * TC, :] - mrow).astype(_BF16)
        vw = vt_scr[pl.ds(st, 24), c * TC:(c + 1) * TC]
        vw = jnp.where(rows24c == r1, jnp.ones_like(vw), vw)
        oc = jnp.dot(vw, p, preferred_element_type=_F32)
        return oc if o is None else o + oc

    def finalize(up, o):
        upc = jnp.maximum(up, 0)
        st, off, r1 = head_rows(upc & (H - 1))
        q0 = pl.multiple_of((upc >> 5) * TQ, TQ)
        l = jnp.sum(jnp.where(rows24q == r1, o, 0.0), axis=0, keepdims=True)
        o = o * (1.0 / l)
        omask = (rows24q >= off) & (rows24q < off + DH) & (up >= 0)
        pltpu.store(ot_scr.at[pl.ds(st, 24), pl.ds(q0, TQ)], o, mask=omask)

    def lagging(up, par_p):
        stp, _, r1p = head_rows(jnp.maximum(up, 0) & (H - 1))
        op = oacc[...]
        mp = mbuf[par_p]
        steps = []
        for c in range(LAG):
            steps.append((stp, r1p, NC - LAG + c, par_p, mp))
        return op, steps

    def step(u, par, extras=(), no_qk=False):
        st, off, r1 = head_rows(u & (H - 1))
        t0 = tile_of(u + 1)
        op, lag_steps = lagging(u - 1, 1 - par)
        mrow = jnp.max(mpart[par], axis=0, keepdims=True)
        if not no_qk:
            qm = qm_scr[...] if par == 0 else qk_w(u + 1)
        m = None
        o = None
        for c in range(NC):
            if not no_qk:
                m = qk_c(qm, t0, c, 1 - par, m)
            if c < LAG:
                op = pv_c(*lag_steps[c], op)
                if c == LAG - 1:
                    finalize(u - 1, op)
            else:
                o = pv_c(st, r1, c - LAG, par, mrow, o)
            if c == 6 and par == 1 and not no_qk:
                qm_scr[...] = qk_w(u + 2)
            for pos, fn in extras:
                if pos == par * NC + c:
                    fn()
        mbuf[par] = mrow
        if not no_qk:
            mpart[1 - par] = m
        oacc[...] = o

    qm0 = qk_w(jnp.int32(0))
    qm_scr[...] = qk_w(jnp.int32(1))
    m0 = None
    for c in range(NC):
        m0 = qk_c(qm0, tile_of(jnp.int32(0)), c, 0, m0)
    mpart[0] = m0
    sbuf[1, (NC - LAG) * TC:NC * TC, :] = jnp.zeros((LAG * TC, TQ), _F32)
    mbuf[1] = jnp.zeros((1, TQ), _F32)
    oacc[...] = jnp.ones((24, TQ), _F32)

    out_copies = []

    def start_out(rows, cols, k):
        cp = pltpu.make_async_copy(out_scr.at[rows[0]:rows[1], cols[0]:cols[1]],
                                   out_hbm.at[rows[0]:rows[1], cols[0]:cols[1]],
                                   out_sems.at[k])
        cp.start()
        out_copies.append(cp)

    def out_proj_tile(q0):
        ob = ot_scr[:, q0:q0 + 128].astype(_BF16)
        bt = jnp.dot(wo_scr[...], ob, preferred_element_type=_F32).astype(_BF16)
        bt = jnp.concatenate([jnp.zeros((64, 128), _BF16), bt], axis=0)
        b = bt.T
        out_scr[q0:q0 + 128, 640:1152] = b[:, 128:640]
        out_scr[q0:q0 + 128, D:640] = b[:, 64:128]

    def out_proj(qb):
        for j in range(TQ // 128):
            out_proj_tile(qb * TQ + 128 * j)

    for qb in range(NQ):
        def heads_body(i, c2, qb=qb):
            u = qb * H + 2 * i
            extras = a_stages[qb](i)
            step(u, 0, extras)
            step(u + 1, 1, extras)
            return c2

        if qb < NQ - 1:
            jax.lax.fori_loop(0, H // 2, heads_body, 0)
            if qb >= 1:
                out_proj(qb - 1)
                start_out(((qb - 1) * TQ, qb * TQ), (640, 1152), qb - 1)
        else:
            jax.lax.fori_loop(0, H // 2 - 1, heads_body, 0)
            il = jnp.int32(H // 2 - 1)
            extras = a_stages[qb](il)
            step(jnp.int32(U - 2), 0, extras)
            last_extras = [(NC + 3 + 3 * j,
                            functools.partial(out_proj_tile, (qb - 1) * TQ + 128 * j))
                           for j in range(TQ // 128)]
            step(jnp.int32(U - 1), 1, list(extras) + last_extras, no_qk=True)
            start_out((0, 2 * TQ), (512, 640), NQ)
            start_out(((qb - 1) * TQ, qb * TQ), (512, 1152), qb - 1)
    op, lag_steps = lagging(jnp.int32(U - 1), 1)
    for c in range(LAG):
        op = pv_c(*lag_steps[c], op)
    finalize(jnp.int32(U - 1), op)
    for j in range(TQ // 128):
        q0 = (NQ - 1) * TQ + 128 * j
        out_proj_tile(q0)
        start_out((q0, q0 + 128), (512, 1152), NQ + 1 + j)
    for j in range(16):
        a_copy(128 * j, j).wait()
    for cp in out_copies:
        cp.wait()


@jax.jit
def pallas_concat_heads__spectral_gfnet__mha_block__prompt_kernel(
    A_x: jax.Array,
    A_w_r: jax.Array,
    A_w_i: jax.Array,
    B_x: jax.Array,
    B_wqkv: jax.Array,
    B_wo: jax.Array,
):
    xat = A_x.reshape(S, D).T
    xbt = B_x.reshape(S, D).T
    wrt = A_w_r.T
    wit = A_w_i.T
    mf = jnp.asarray(_MF, dtype=_BF16)
    mi = jnp.asarray(_MI, dtype=_BF16)
    gt = jnp.asarray(_GT, dtype=_BF16)
    gi = jnp.asarray(_GI, dtype=_BF16)

    any_spec = pl.BlockSpec(memory_space=pl.ANY)
    out = pl.pallas_call(
        _kernel,
        out_shape=jax.ShapeDtypeStruct((S, 2 * D), _BF16),
        in_specs=[any_spec] * 10,
        out_specs=any_spec,
        scratch_shapes=[
            pltpu.VMEM((D, S), _BF16),
            pltpu.VMEM((DF, S), _BF16),
            pltpu.VMEM((DF, S), _BF16),
            pltpu.VMEM((D, S), _BF16),
            pltpu.VMEM((D, 3 * D), _BF16),
            pltpu.VMEM((D, D), _BF16),
            pltpu.VMEM((5, 128, 128), _BF16),
            pltpu.VMEM((5, 128, 128), _BF16),
            pltpu.VMEM((16, 128, 256), _BF16),
            pltpu.VMEM((16, 128, 256), _BF16),
            pltpu.VMEM((S, 2 * D), _BF16),
            pltpu.SemaphoreType.DMA((8,)),
            pltpu.SemaphoreType.DMA((NQ + 1 + TQ // 128,)),
            pltpu.SemaphoreType.DMA((16,)),
            pltpu.SemaphoreType.DMA((3,)),
            pltpu.SemaphoreType.DMA((S // RC,)),
            pltpu.VMEM((S, LW), _BF16),
            pltpu.VMEM((LW, S), _BF16),
            pltpu.VMEM((D, S), _F32),
            pltpu.VMEM((D, S), _F32),
            pltpu.VMEM((2, S, TQ), _F32),
            pltpu.VMEM((2, 1, TQ), _F32),
            pltpu.VMEM((QR, D), _BF16),
            pltpu.VMEM((QR, D), _BF16),
            pltpu.VMEM((D, D), _BF16),
            pltpu.VMEM((D, D), _BF16),
            pltpu.VMEM((2 * NR, S), _F32),
            pltpu.VMEM((2 * NR, S), _F32),
            pltpu.VMEM((6, S, 128), _F32),
            pltpu.VMEM((2, 384, 128), _F32),
            pltpu.VMEM((2 * NR, S), _F32),
            pltpu.VMEM((128, TQ), _BF16),
            pltpu.VMEM((2, 8, TQ), _F32),
            pltpu.VMEM((24, TQ), _F32),
        ],
        compiler_params=pltpu.CompilerParams(vmem_limit_bytes=100 * 1024 * 1024),
    )(xat, wrt, wit, xbt, B_wqkv, B_wo, mf, mi, gt, gi)
    return out.reshape(1, S, 2 * D)
```

```python
import functools
import math

import numpy as np
import jax
import jax.numpy as jnp
import jax.experimental.pallas as pl
import jax.experimental.pallas.tpu as pltpu

S = 2048
D = 576
H = 32
DH = D // H
DF = D // 2 + 1
LW = 640
TQ = 512
TC = 128
RC = 256
NQ = S // TQ
NC = S // TC
LAG = 3
REP = 4
QR = 592
HPT = 7
NR = 296
NG = NR // 8

_F32 = jnp.float32
_BF16 = jnp.bfloat16


def _dft_tables():
    n2 = np.arange(64)
    mf = np.zeros((5, 128, 128), np.float64)
    mi = np.zeros((5, 128, 128), np.float64)
    for k1 in range(1, 5):
        for part, base in ((0, k1), (1, 9 - k1)):
            sg = 1.0 if part == 0 else -1.0
            for j in range(32):
                k = base + 9 * j
                ang = 2.0 * np.pi * ((n2 * k) % D) / D
                c, s = np.cos(ang), np.sin(ang)
                rr = 32 * part + j
                ri = 64 + 32 * part + j
                mf[k1 - 1, rr, :64] = c
                mf[k1 - 1, rr, 64:] = sg * s
                mf[k1 - 1, ri, :64] = -s
                mf[k1 - 1, ri, 64:] = sg * c
                f = 2.0 / (S * D)
                mi[k1 - 1, :64, rr] = f * c
                mi[k1 - 1, :64, ri] = -f * s
                mi[k1 - 1, 64:, rr] = f * sg * s
                mi[k1 - 1, 64:, ri] = f * sg * c
    for j in range(33):
        k = 9 * j
        ang = 2.0 * np.pi * ((n2 * k) % D) / D
        c, s = np.cos(ang), np.sin(ang)
        mf[4, j, :64] = c
        mf[4, 40 + j, :64] = -s
        f = (1.0 if j in (0, 32) else 2.0) / (S * D)
        mi[4, :64, j] = f * c
        if j not in (0, 32):
            mi[4, :64, 40 + j] = -f * s
    m2 = np.arange(128)
    gt = np.zeros((16, 128, 256), np.float64)
    gi = np.zeros((16, 128, 256), np.float64)
    for k1 in range(16):
        ang = -2.0 * np.pi * (np.outer(k1 + 16 * m2, m2) % S) / S
        gt[k1, :, :128] = np.cos(ang).T
        gt[k1, :, 128:] = np.sin(ang).T
        gi[k1, :, :128] = np.cos(ang)
        gi[k1, :, 128:] = np.sin(ang)
    return mf, mi, gt, gi


_MF, _MI, _GT, _GI = _dft_tables()
_C9 = [[math.cos(2.0 * math.pi * j * k / 9.0) for k in range(5)] for j in range(5)]
_S9 = [[math.sin(2.0 * math.pi * j * k / 9.0) for k in range(5)] for j in range(5)]


def _cmul_w16(z, e, sign):
    re, im = z
    e = e % 16
    if e == 0:
        return z
    c = math.cos(2.0 * math.pi * e / 16.0)
    s = sign * math.sin(2.0 * math.pi * e / 16.0)
    if e == 4:
        return (-im, re) if sign > 0 else (im, -re)
    if e % 4 == 2:
        r = math.sqrt(0.5)
        a = re * r
        b = im * r
        cr = 1.0 if c > 0 else -1.0
        sr = 1.0 if s > 0 else -1.0
        nre = (a if cr > 0 else -a) - (b if sr > 0 else -b)
        nim = (a if sr > 0 else -a) + (b if cr > 0 else -b)
        return nre, nim
    return re * c - im * s, re * s + im * c


def _dft4(x0, x1, x2, x3, sign):
    e = (x0[0] + x2[0], x0[1] + x2[1])
    f = (x0[0] - x2[0], x0[1] - x2[1])
    g = (x1[0] + x3[0], x1[1] + x3[1])
    h = (x1[0] - x3[0], x1[1] - x3[1])
    y0 = (e[0] + g[0], e[1] + g[1])
    y2 = (e[0] - g[0], e[1] - g[1])
    if sign > 0:
        y1 = (f[0] - h[1], f[1] + h[0])
        y3 = (f[0] + h[1], f[1] - h[0])
    else:
        y1 = (f[0] + h[1], f[1] - h[0])
        y3 = (f[0] - h[1], f[1] + h[0])
    return y0, y1, y2, y3


def _dft16(xs, sign):
    t = [_dft4(xs[b], xs[4 + b], xs[8 + b], xs[12 + b], sign) for b in range(4)]
    t = [[_cmul_w16(t[b][c], b * c, sign) for c in range(4)] for b in range(4)]
    out = [None] * 16
    for c in range(4):
        ys = _dft4(t[0][c], t[1][c], t[2][c], t[3][c], sign)
        for dd in range(4):
            out[c + 4 * dd] = ys[dd]
    return out


def _lin(terms):
    acc = None
    for cf, arr in terms:
        if abs(cf) < 1e-12:
            continue
        if abs(cf - 1.0) < 1e-12:
            acc = arr if acc is None else acc + arr
        elif abs(cf + 1.0) < 1e-12:
            acc = -arr if acc is None else acc - arr
        else:
            t = arr * cf
            acc = t if acc is None else acc + t
    return acc


def _kernel(xat_hbm, wrt_hbm, wit_hbm, xbt_hbm, wqkv_hbm, wo_hbm,
            mf_hbm, mi_hbm, gt_hbm, gi_hbm,
            out_hbm,
            xat_ref, wrt_ref, wit_ref, xbt_ref, wqkv_ref, wo_ref,
            mf_ref, mi_ref, gt_ref, gi_ref,
            out_scr, in_sems, out_sems, a_sems, w_sems, x_sems,
            k_scr, qt_scr, vt_scr, ot_scr, sbuf, mbuf,
            wk_scr, wqt_scr, wvt_scr, wo_scr,
            y_scr, y2_scr, w_scr, wt_scr, wp_scr, qm_scr, mpart, oacc):
    srcs = (xat_hbm, mf_hbm, wrt_hbm, wit_hbm, wo_hbm, gt_hbm, gi_hbm, mi_hbm)
    dsts = (xat_ref, mf_ref, wrt_ref, wit_ref, wo_ref, gt_ref, gi_ref, mi_ref)
    copies = [pltpu.make_async_copy(s, d, in_sems.at[i])
              for i, (s, d) in enumerate(zip(srcs, dsts))]
    wcols = ((0, 640), (640, 1280), (1280, 3 * D))
    wcopies = [pltpu.make_async_copy(wqkv_hbm.at[:, a:b], wqkv_ref.at[:, a:b], w_sems.at[i])
               for i, (a, b) in enumerate(wcols)]

    def x_copy(c0, i):
        return pltpu.make_async_copy(xbt_hbm.at[:, pl.ds(c0, RC)],
                                     xbt_ref.at[:, pl.ds(c0, RC)], x_sems.at[i])

    wcopies[0].start()
    wcopies[1].start()

    wcopies[0].wait()
    wcopies[2].start()
    x_copy(0, 0).start()
    for t in range(5):
        n = 128 if t < 4 else QR - 512
        wqt_scr[128 * t:128 * t + n, :] = wqkv_ref[:, 126 * t:126 * t + 128].T[0:n]
    wcopies[1].wait()
    for i in range(1, S // RC):
        x_copy(i * RC, i).start()
    for t in range(5):
        n = 128 if t < 4 else QR - 512
        wk_scr[128 * t:128 * t + n, :] = wqkv_ref[:, D + 126 * t:D + 126 * t + 128].T[0:n]
    wcopies[2].wait()
    wvt_scr[...] = wqkv_ref[:, 2 * D:3 * D].T

    qscale = (DH ** -0.5) * math.log2(math.e)
    for cp in copies:
        cp.start()

    def proj(i):
        r0 = pl.multiple_of(i * RC, RC)
        x_copy(r0, i).wait()
        xt = xbt_ref[:, pl.ds(r0, RC)]
        kt = jnp.dot(wk_scr[...], xt, preferred_element_type=_F32).astype(_BF16)
        kt = jnp.concatenate([kt, jnp.zeros((LW - QR, RC), _BF16)], axis=0)
        k_scr[pl.ds(r0, RC), :] = kt.T
        qt = jnp.dot(wqt_scr[...], xt, preferred_element_type=_F32)
        qt_scr[0:QR, pl.ds(r0, RC)] = (qt * qscale).astype(_BF16)
        vt = jnp.dot(wvt_scr[...], xt, preferred_element_type=_F32)
        vt_scr[:, pl.ds(r0, RC)] = vt.astype(_BF16).astype(_F32)

    def dfwd_tile(l0):
        xt = xat_ref[:, pl.ds(l0, 128)].astype(_F32)
        xb = [xt[64 * n:64 * (n + 1)] for n in range(9)]
        u = [None] + [xb[j] + xb[9 - j] for j in range(1, 5)]
        v = [None] + [xb[j] - xb[9 - j] for j in range(1, 5)]
        for k in range(1, 5):
            ar = _lin([(1.0, xb[0])] + [(_C9[j][k], u[j]) for j in range(1, 5)])
            ai = _lin([(-_S9[j][k], v[j]) for j in range(1, 5)])
            a = jnp.concatenate([ar, ai], axis=0).astype(_BF16)
            o = jnp.dot(mf_ref[k - 1], a, preferred_element_type=_F32)
            y_scr[64 * (k - 1):64 * k, pl.ds(l0, 128)] = o[:64]
            y_scr[NR + 64 * (k - 1):NR + 64 * k, pl.ds(l0, 128)] = o[64:]
        a0 = (xb[0] + (u[1] + u[2]) + (u[3] + u[4])).astype(_BF16)
        o = jnp.dot(mf_ref[4, 0:80, 0:64], a0, preferred_element_type=_F32)
        y_scr[256:NR, pl.ds(l0, 128)] = o[:40]
        y_scr[NR + 256:2 * NR, pl.ds(l0, 128)] = o[40:]

    def wnat_chunk(r0):
        wr = wrt_ref[:, pl.ds(r0, 256)].T.astype(_F32)
        wi = wit_ref[:, pl.ds(r0, 256)].T.astype(_F32)
        z = jnp.zeros((256, 128), _F32)
        for p, w in ((0, wr), (1, wi)):
            w_scr[3 * p + 0, pl.ds(r0, 256), :] = w[:, 0:128]
            w_scr[3 * p + 1, pl.ds(r0, 256), :] = w[:, 128:256]
            w_scr[3 * p + 2, pl.ds(r0, 256), :] = z
            w_scr[3 * p + 2, pl.ds(r0, 256), 0:33] = w[:, 256:289]

    def proj_body1(i, carry):
        proj(i)
        return carry

    jax.lax.fori_loop(0, 4, proj_body1, 0)

    for i in range(0, 4):
        copies[i].wait()

    def proj_body2(i, carry):
        proj(4 + i)
        for j in range(4):
            dfwd_tile(pl.multiple_of(i * 512 + j * 128, 128))
        for j in range(2):
            wnat_chunk(pl.multiple_of(i * 512 + j * 256, 256))
        return carry

    jax.lax.fori_loop(0, 4, proj_body2, 0)

    for i in range(4, 8):
        copies[i].wait()
    wo_scr[...] = wo_ref[...].T

    def bfly_group(g, sign):
        r0 = pl.multiple_of(jnp.minimum(g, NG - 1) * 8, 8)
        xs = [(y_scr[pl.ds(r0, 8), 128 * n:128 * (n + 1)],
               y_scr[pl.ds(NR + r0, 8), 128 * n:128 * (n + 1)]) for n in range(16)]
        ys = _dft16(xs, sign)
        for n in range(16):
            y2_scr[pl.ds(r0, 8), 128 * n:128 * (n + 1)] = ys[n][0]
            y2_scr[pl.ds(NR + r0, 8), 128 * n:128 * (n + 1)] = ys[n][1]

    def wperm_slice(k1s):
        l0 = pl.multiple_of(k1s * 128, 128)
        for p in range(2):
            for t in range(3):
                blk = w_scr[3 * p + t, pl.ds(k1s, 128, stride=16), :]
                wt_scr[p, 128 * t:128 * (t + 1), :] = blk.T
            for k in range(1, 5):
                wp_scr[NR * p + 64 * (k - 1):NR * p + 64 * (k - 1) + 32, pl.ds(l0, 128)] = (
                    wt_scr[p, pl.ds(k, 32, stride=9), :])
                wp_scr[NR * p + 64 * (k - 1) + 32:NR * p + 64 * k, pl.ds(l0, 128)] = (
                    wt_scr[p, pl.ds(9 - k, 32, stride=9), :])
            wp_scr[NR * p + 256:NR * (p + 1), pl.ds(l0, 128)] = (
                wt_scr[p, pl.ds(0, 40, stride=9), :])

    def bfly_slots(ii, sign):
        i, r = ii
        offs = ((0, 1, 2), (3, 4, 5), (6, 7), (8, 9))[r]
        pos = (1, 10, 20)
        return [(pos[n], functools.partial(bfly_group, 10 * i + o, sign))
                for n, o in enumerate(offs)]

    def stage_bfly_fwd(ii):
        return bfly_slots(ii, -1) + [(16, lambda: wperm_slice(ii[0] * REP + ii[1]))]

    def stage_bfly_inv(ii):
        return bfly_slots(ii, 1)

    def stage_smid(ii):
        k1s = ii[0] * REP + ii[1]
        l0 = pl.multiple_of(k1s * 128, 128)
        st = {}

        def part_a():
            st["p"] = jnp.dot(y2_scr[:, pl.ds(l0, 128)], gt_ref[k1s],
                              preferred_element_type=_F32)

        def part_b():
            p = st["p"]
            xr = p[:NR, :128] - p[NR:, 128:]
            xi = p[NR:, :128] + p[:NR, 128:]
            wpr = wp_scr[0:NR, pl.ds(l0, 128)]
            wpi = wp_scr[NR:2 * NR, pl.ds(l0, 128)]
            z = jnp.concatenate([xr * wpr - xi * wpi, xr * wpi + xi * wpr], axis=0)
            st["q"] = jnp.dot(z, gi_ref[k1s], preferred_element_type=_F32)

        def part_c():
            q = st["q"]
            y_scr[0:NR, pl.ds(l0, 128)] = q[:NR, :128] + q[NR:, 128:]
            y_scr[NR:2 * NR, pl.ds(l0, 128)] = q[NR:, :128] - q[:NR, 128:]

        return [(2, part_a), (12, part_b), (22, part_c)]

    def a_copy(r0, j):
        return pltpu.make_async_copy(out_scr.at[pl.ds(r0, 128), 0:512],
                                     out_hbm.at[pl.ds(r0, 128), 0:512], a_sems.at[j])

    def stage_dinv(ii):
        j = ii[0] * REP + ii[1]
        l0 = pl.multiple_of(j * 128, 128)
        st = {}

        def part_a():
            cs = []
            for k in range(1, 5):
                zz = jnp.concatenate(
                    [y2_scr[64 * (k - 1):64 * k, pl.ds(l0, 128)],
                     y2_scr[NR + 64 * (k - 1):NR + 64 * k, pl.ds(l0, 128)]],
                    axis=0).astype(_BF16)
                cs.append(jnp.dot(mi_ref[k - 1], zz, preferred_element_type=_F32))
            zz = jnp.concatenate(
                [y2_scr[256:NR, pl.ds(l0, 128)],
                 y2_scr[NR + 256:2 * NR, pl.ds(l0, 128)]], axis=0).astype(_BF16)
            st["c0"] = jnp.dot(mi_ref[4, 0:64, 0:80], zz, preferred_element_type=_F32)
            st["cs"] = cs

        def part_b():
            c0 = st["c0"]
            cr = [None] + [c[:64] for c in st["cs"]]
            ci = [None] + [c[64:] for c in st["cs"]]
            ys = [None] * 9
            ys[0] = c0 + (cr[1] + cr[2]) + (cr[3] + cr[4])
            for n in range(1, 5):
                e = _lin([(1.0, c0)] + [(_C9[n][k], cr[k]) for k in range(1, 5)])
                o = _lin([(_S9[n][k], ci[k]) for k in range(1, 5)])
                ys[n] = e - o
                ys[9 - n] = e + o
            yt = jnp.concatenate(ys, axis=0).astype(_BF16)
            out_scr[pl.ds(l0, 128), 0:D] = yt.T

        def part_c():
            a_copy(l0, j).start()

        return [(2, part_a), (12, part_b), (2 * NC - 1, part_c)]

    a_stages = (stage_bfly_fwd, stage_smid, stage_bfly_inv, stage_dinv)

    U = NQ * H
    rows128 = jax.lax.broadcasted_iota(jnp.int32, (128, TQ), 0)
    rows24q = jax.lax.broadcasted_iota(jnp.int32, (24, TQ), 0)
    rows24c = jax.lax.broadcasted_iota(jnp.int32, (24, TC), 0)

    def div7(h):
        return (h * 37) >> 8

    def tile_of(u):
        h = jnp.minimum(u, U - 1) & (H - 1)
        return pl.multiple_of(div7(h) * 128, 128)

    def qk_w(u):
        u = jnp.minimum(u, U - 1)
        qb = u >> 5
        h = u & (H - 1)
        j = h - div7(h) * HPT
        q0 = pl.multiple_of(qb * TQ, TQ)
        qt = qt_scr[pl.ds(tile_of(u), 128), pl.ds(q0, TQ)]
        mask = (rows128 >= j * DH) & (rows128 < (j + 1) * DH)
        return jnp.where(mask, qt, jnp.zeros_like(qt))

    def qk_c(qm, t0, c, slot, m):
        kt = k_scr[c * TC:(c + 1) * TC, pl.ds(t0, 128)]
        s = jnp.dot(kt, qm, preferred_element_type=_F32)
        sbuf[slot, c * TC:(c + 1) * TC, :] = s
        mc = jnp.max(s.reshape(TC // 8, 8, TQ), axis=0)
        return mc if m is None else jnp.maximum(m, mc)

    def head_rows(h):
        st = pl.multiple_of(((h * DH) >> 3) * 8, 8)
        off = h * DH - st
        return st, off, jnp.where(off == 6, 0, off + DH)

    def pv_c(st, r1, c, slot, mrow, o):
        p = jnp.exp2(sbuf[slot, c * TC:(c + 1) * TC, :] - mrow).astype(_BF16)
        vw = vt_scr[pl.ds(st, 24), c * TC:(c + 1) * TC]
        vw = jnp.where(rows24c == r1, jnp.ones_like(vw), vw)
        oc = jnp.dot(vw, p, preferred_element_type=_F32)
        return oc if o is None else o + oc

    def finalize(up, o):
        upc = jnp.maximum(up, 0)
        st, off, r1 = head_rows(upc & (H - 1))
        q0 = pl.multiple_of((upc >> 5) * TQ, TQ)
        l = jnp.sum(jnp.where(rows24q == r1, o, 0.0), axis=0, keepdims=True)
        o = o * (1.0 / l)
        omask = (rows24q >= off) & (rows24q < off + DH) & (up >= 0)
        pltpu.store(ot_scr.at[pl.ds(st, 24), pl.ds(q0, TQ)], o, mask=omask)

    def lagging(up, par_p):
        stp, _, r1p = head_rows(jnp.maximum(up, 0) & (H - 1))
        op = oacc[...]
        mp = mbuf[par_p]
        steps = []
        for c in range(LAG):
            steps.append((stp, r1p, NC - LAG + c, par_p, mp))
        return op, steps

    def step(u, par, extras=(), no_qk=False, first=False, last=False):
        st, off, r1 = head_rows(u & (H - 1))
        t0 = tile_of(u + 1)
        op, lag_steps = lagging(u - 1, 1 - par)
        mrow = jnp.max(mpart[par], axis=0, keepdims=True)
        if not no_qk:
            qm = qm_scr[...] if first else qk_w(u + 1)
        m = None
        o = None
        for c in range(NC):
            if not no_qk:
                m = qk_c(qm, t0, c, 1 - par, m)
            if c < LAG:
                op = pv_c(*lag_steps[c], op)
                if c == LAG - 1:
                    finalize(u - 1, op)
            else:
                o = pv_c(st, r1, c - LAG, par, mrow, o)
            if c == 6 and last:
                qm_scr[...] = qk_w(u + 2)
            for pos, fn in extras:
                if pos == par * NC + c:
                    fn()
        mbuf[par] = mrow
        if not no_qk:
            mpart[1 - par] = m
        oacc[...] = o

    qm0 = qk_w(jnp.int32(0))
    qm_scr[...] = qk_w(jnp.int32(1))
    m0 = None
    for c in range(NC):
        m0 = qk_c(qm0, tile_of(jnp.int32(0)), c, 0, m0)
    mpart[0] = m0
    sbuf[1, (NC - LAG) * TC:NC * TC, :] = jnp.zeros((LAG * TC, TQ), _F32)
    mbuf[1] = jnp.zeros((1, TQ), _F32)
    oacc[...] = jnp.ones((24, TQ), _F32)

    out_copies = []

    def start_out(rows, cols, k):
        cp = pltpu.make_async_copy(out_scr.at[rows[0]:rows[1], cols[0]:cols[1]],
                                   out_hbm.at[rows[0]:rows[1], cols[0]:cols[1]],
                                   out_sems.at[k])
        cp.start()
        out_copies.append(cp)

    def out_proj_tile(q0):
        ob = ot_scr[:, q0:q0 + 128].astype(_BF16)
        bt = jnp.dot(wo_scr[...], ob, preferred_element_type=_F32).astype(_BF16)
        bt = jnp.concatenate([jnp.zeros((64, 128), _BF16), bt], axis=0)
        b = bt.T
        out_scr[q0:q0 + 128, 640:1152] = b[:, 128:640]
        out_scr[q0:q0 + 128, D:640] = b[:, 64:128]

    def out_proj(qb):
        for j in range(TQ // 128):
            out_proj_tile(qb * TQ + 128 * j)

    for qb in range(NQ):
        def heads_body(i, c2, qb=qb, rep=REP):
            for r in range(rep):
                ii = i * REP + r
                u = qb * H + 2 * ii
                extras = a_stages[qb]((i, r))
                step(u, 0, extras, first=(r == 0))
                step(u + 1, 1, extras, last=(r == rep - 1))
            return c2

        if qb < NQ - 1:
            jax.lax.fori_loop(0, H // (2 * REP), heads_body, 0)
            if qb >= 1:
                out_proj(qb - 1)
                start_out(((qb - 1) * TQ, qb * TQ), (640, 1152), qb - 1)
        else:
            jax.lax.fori_loop(0, H // (2 * REP) - 1, heads_body, 0)
            if REP > 1:
                heads_body(jnp.int32(H // (2 * REP) - 1), 0, rep=REP - 1)
            extras = a_stages[qb]((jnp.int32(H // (2 * REP) - 1), REP - 1))
            step(jnp.int32(U - 2), 0, extras, first=True)
            last_extras = [(NC + 3 + 3 * j,
                            functools.partial(out_proj_tile, (qb - 1) * TQ + 128 * j))
                           for j in range(TQ // 128)]
            step(jnp.int32(U - 1), 1, list(extras) + last_extras, no_qk=True)
            start_out((0, 2 * TQ), (512, 640), NQ)
            start_out(((qb - 1) * TQ, qb * TQ), (512, 1152), qb - 1)
    op, lag_steps = lagging(jnp.int32(U - 1), 1)
    for c in range(LAG):
        op = pv_c(*lag_steps[c], op)
    finalize(jnp.int32(U - 1), op)
    for j in range(TQ // 128):
        q0 = (NQ - 1) * TQ + 128 * j
        out_proj_tile(q0)
        start_out((q0, q0 + 128), (512, 1152), NQ + 1 + j)
    for j in range(16):
        a_copy(128 * j, j).wait()
    for cp in out_copies:
        cp.wait()


@jax.jit
def pallas_concat_heads__spectral_gfnet__mha_block__prompt_kernel(
    A_x: jax.Array,
    A_w_r: jax.Array,
    A_w_i: jax.Array,
    B_x: jax.Array,
    B_wqkv: jax.Array,
    B_wo: jax.Array,
):
    xat = A_x.reshape(S, D).T
    xbt = B_x.reshape(S, D).T
    wrt = A_w_r.T
    wit = A_w_i.T
    mf = jnp.asarray(_MF, dtype=_BF16)
    mi = jnp.asarray(_MI, dtype=_BF16)
    gt = jnp.asarray(_GT, dtype=_BF16)
    gi = jnp.asarray(_GI, dtype=_BF16)

    any_spec = pl.BlockSpec(memory_space=pl.ANY)
    out = pl.pallas_call(
        _kernel,
        out_shape=jax.ShapeDtypeStruct((S, 2 * D), _BF16),
        in_specs=[any_spec] * 10,
        out_specs=any_spec,
        scratch_shapes=[
            pltpu.VMEM((D, S), _BF16),
            pltpu.VMEM((DF, S), _BF16),
            pltpu.VMEM((DF, S), _BF16),
            pltpu.VMEM((D, S), _BF16),
            pltpu.VMEM((D, 3 * D), _BF16),
            pltpu.VMEM((D, D), _BF16),
            pltpu.VMEM((5, 128, 128), _BF16),
            pltpu.VMEM((5, 128, 128), _BF16),
            pltpu.VMEM((16, 128, 256), _BF16),
            pltpu.VMEM((16, 128, 256), _BF16),
            pltpu.VMEM((S, 2 * D), _BF16),
            pltpu.SemaphoreType.DMA((8,)),
            pltpu.SemaphoreType.DMA((NQ + 1 + TQ // 128,)),
            pltpu.SemaphoreType.DMA((16,)),
            pltpu.SemaphoreType.DMA((3,)),
            pltpu.SemaphoreType.DMA((S // RC,)),
            pltpu.VMEM((S, LW), _BF16),
            pltpu.VMEM((LW, S), _BF16),
            pltpu.VMEM((D, S), _F32),
            pltpu.VMEM((D, S), _F32),
            pltpu.VMEM((2, S, TQ), _F32),
            pltpu.VMEM((2, 1, TQ), _F32),
            pltpu.VMEM((QR, D), _BF16),
            pltpu.VMEM((QR, D), _BF16),
            pltpu.VMEM((D, D), _BF16),
            pltpu.VMEM((D, D), _BF16),
            pltpu.VMEM((2 * NR, S), _F32),
            pltpu.VMEM((2 * NR, S), _F32),
            pltpu.VMEM((6, S, 128), _F32),
            pltpu.VMEM((2, 384, 128), _F32),
            pltpu.VMEM((2 * NR, S), _F32),
            pltpu.VMEM((128, TQ), _BF16),
            pltpu.VMEM((2, 8, TQ), _F32),
            pltpu.VMEM((24, TQ), _F32),
        ],
        compiler_params=pltpu.CompilerParams(vmem_limit_bytes=100 * 1024 * 1024),
    )(xat, wrt, wit, xbt, B_wqkv, B_wo, mf, mi, gt, gi)
    return out.reshape(1, S, 2 * D)
```

```python
import functools
import math

import numpy as np
import jax
import jax.numpy as jnp
import jax.experimental.pallas as pl
import jax.experimental.pallas.tpu as pltpu

S = 2048
D = 576
H = 32
DH = D // H
DF = D // 2 + 1
LW = 640
TQ = 512
TC = 128
RC = 256
NQ = S // TQ
NC = S // TC
LAG = 3
REP = 4
QR = 592
HPT = 7
NR = 296
NG = NR // 8

_F32 = jnp.float32
_BF16 = jnp.bfloat16


def _dft_tables():
    n2 = np.arange(64)
    mf = np.zeros((5, 128, 128), np.float64)
    mi = np.zeros((5, 128, 128), np.float64)
    for k1 in range(1, 5):
        for part, base in ((0, k1), (1, 9 - k1)):
            sg = 1.0 if part == 0 else -1.0
            for j in range(32):
                k = base + 9 * j
                ang = 2.0 * np.pi * ((n2 * k) % D) / D
                c, s = np.cos(ang), np.sin(ang)
                rr = 32 * part + j
                ri = 64 + 32 * part + j
                mf[k1 - 1, rr, :64] = c
                mf[k1 - 1, rr, 64:] = sg * s
                mf[k1 - 1, ri, :64] = -s
                mf[k1 - 1, ri, 64:] = sg * c
                f = 2.0 / (S * D)
                mi[k1 - 1, :64, rr] = f * c
                mi[k1 - 1, :64, ri] = -f * s
                mi[k1 - 1, 64:, rr] = f * sg * s
                mi[k1 - 1, 64:, ri] = f * sg * c
    for j in range(33):
        k = 9 * j
        ang = 2.0 * np.pi * ((n2 * k) % D) / D
        c, s = np.cos(ang), np.sin(ang)
        mf[4, j, :64] = c
        mf[4, 40 + j, :64] = -s
        f = (1.0 if j in (0, 32) else 2.0) / (S * D)
        mi[4, :64, j] = f * c
        if j not in (0, 32):
            mi[4, :64, 40 + j] = -f * s
    m2 = np.arange(128)
    gt = np.zeros((16, 128, 256), np.float64)
    gi = np.zeros((16, 128, 256), np.float64)
    for k1 in range(16):
        ang = -2.0 * np.pi * (np.outer(k1 + 16 * m2, m2) % S) / S
        gt[k1, :, :128] = np.cos(ang).T
        gt[k1, :, 128:] = np.sin(ang).T
        gi[k1, :, :128] = np.cos(ang)
        gi[k1, :, 128:] = np.sin(ang)
    return mf, mi, gt, gi


_MF, _MI, _GT, _GI = _dft_tables()
_C9 = [[math.cos(2.0 * math.pi * j * k / 9.0) for k in range(5)] for j in range(5)]
_S9 = [[math.sin(2.0 * math.pi * j * k / 9.0) for k in range(5)] for j in range(5)]


def _cmul_w16(z, e, sign):
    re, im = z
    e = e % 16
    if e == 0:
        return z
    c = math.cos(2.0 * math.pi * e / 16.0)
    s = sign * math.sin(2.0 * math.pi * e / 16.0)
    if e == 4:
        return (-im, re) if sign > 0 else (im, -re)
    if e % 4 == 2:
        r = math.sqrt(0.5)
        a = re * r
        b = im * r
        cr = 1.0 if c > 0 else -1.0
        sr = 1.0 if s > 0 else -1.0
        nre = (a if cr > 0 else -a) - (b if sr > 0 else -b)
        nim = (a if sr > 0 else -a) + (b if cr > 0 else -b)
        return nre, nim
    return re * c - im * s, re * s + im * c


def _dft4(x0, x1, x2, x3, sign):
    e = (x0[0] + x2[0], x0[1] + x2[1])
    f = (x0[0] - x2[0], x0[1] - x2[1])
    g = (x1[0] + x3[0], x1[1] + x3[1])
    h = (x1[0] - x3[0], x1[1] - x3[1])
    y0 = (e[0] + g[0], e[1] + g[1])
    y2 = (e[0] - g[0], e[1] - g[1])
    if sign > 0:
        y1 = (f[0] - h[1], f[1] + h[0])
        y3 = (f[0] + h[1], f[1] - h[0])
    else:
        y1 = (f[0] + h[1], f[1] - h[0])
        y3 = (f[0] - h[1], f[1] + h[0])
    return y0, y1, y2, y3


def _dft16(xs, sign):
    t = [_dft4(xs[b], xs[4 + b], xs[8 + b], xs[12 + b], sign) for b in range(4)]
    t = [[_cmul_w16(t[b][c], b * c, sign) for c in range(4)] for b in range(4)]
    out = [None] * 16
    for c in range(4):
        ys = _dft4(t[0][c], t[1][c], t[2][c], t[3][c], sign)
        for dd in range(4):
            out[c + 4 * dd] = ys[dd]
    return out


def _lin(terms):
    acc = None
    for cf, arr in terms:
        if abs(cf) < 1e-12:
            continue
        if abs(cf - 1.0) < 1e-12:
            acc = arr if acc is None else acc + arr
        elif abs(cf + 1.0) < 1e-12:
            acc = -arr if acc is None else acc - arr
        else:
            t = arr * cf
            acc = t if acc is None else acc + t
    return acc


def _kernel(xat_hbm, wrt_hbm, wit_hbm, xbt_hbm, wqkv_hbm, wo_hbm,
            mf_hbm, mi_hbm, gt_hbm, gi_hbm,
            out_hbm,
            xat_ref, wrt_ref, wit_ref, xbt_ref, wqkv_ref, wo_ref,
            mf_ref, mi_ref, gt_ref, gi_ref,
            out_scr, in_sems, out_sems, a_sems, w_sems, x_sems,
            k_scr, qt_scr, vt_scr, ot_scr, sbuf, mbuf,
            wk_scr, wqt_scr, wvt_scr, wo_scr,
            y_scr, y2_scr, w_scr, wt_scr, wp_scr, qm_scr, mpart, oacc):
    srcs = (wrt_hbm, wit_hbm, xat_hbm, mf_hbm, wo_hbm, gt_hbm, gi_hbm, mi_hbm)
    dsts = (wrt_ref, wit_ref, xat_ref, mf_ref, wo_ref, gt_ref, gi_ref, mi_ref)
    copies = [pltpu.make_async_copy(s, d, in_sems.at[i])
              for i, (s, d) in enumerate(zip(srcs, dsts))]
    wcols = ((0, 640), (640, 1280), (1280, 3 * D))
    wcopies = [pltpu.make_async_copy(wqkv_hbm.at[:, a:b], wqkv_ref.at[:, a:b], w_sems.at[i])
               for i, (a, b) in enumerate(wcols)]

    def x_copy(c0, i):
        return pltpu.make_async_copy(xbt_hbm.at[:, pl.ds(c0, RC)],
                                     xbt_ref.at[:, pl.ds(c0, RC)], x_sems.at[i])

    wcopies[0].start()
    x_copy(0, 0).start()
    wcopies[1].start()

    qscale = (DH ** -0.5) * math.log2(math.e)

    def proj_k(r0, xt):
        kt = jnp.dot(wk_scr[...], xt, preferred_element_type=_F32).astype(_BF16)
        kt = jnp.concatenate([kt, jnp.zeros((LW - QR, RC), _BF16)], axis=0)
        k_scr[pl.ds(r0, RC), :] = kt.T

    def proj_q(r0, xt):
        qt = jnp.dot(wqt_scr[...], xt, preferred_element_type=_F32)
        qt_scr[0:QR, pl.ds(r0, RC)] = (qt * qscale).astype(_BF16)

    def proj_v(r0, xt):
        vt = jnp.dot(wvt_scr[...], xt, preferred_element_type=_F32)
        vt_scr[:, pl.ds(r0, RC)] = vt.astype(_BF16).astype(_F32)

    def proj(i):
        r0 = i * RC if isinstance(i, int) else pl.multiple_of(i * RC, RC)
        x_copy(r0, i).wait()
        xt = xbt_ref[:, pl.ds(r0, RC)]
        proj_k(r0, xt)
        proj_q(r0, xt)
        proj_v(r0, xt)

    wcopies[0].wait()
    wcopies[2].start()
    for t in range(5):
        n = 128 if t < 4 else QR - 512
        wqt_scr[128 * t:128 * t + n, :] = wqkv_ref[:, 126 * t:126 * t + 128].T[0:n]
    wcopies[1].wait()
    x_copy(0, 0).wait()
    for i in range(1, S // RC):
        x_copy(i * RC, i).start()
    proj_q(0, xbt_ref[:, 0:RC])
    for t in range(5):
        n = 128 if t < 4 else QR - 512
        wk_scr[128 * t:128 * t + n, :] = wqkv_ref[:, D + 126 * t:D + 126 * t + 128].T[0:n]
    wcopies[2].wait()
    for cp in copies[:4]:
        cp.start()
    proj_k(0, xbt_ref[:, 0:RC])
    wvt_scr[...] = wqkv_ref[:, 2 * D:3 * D].T
    proj_v(0, xbt_ref[:, 0:RC])
    proj(1)

    def dfwd_tile(l0):
        xt = xat_ref[:, pl.ds(l0, 128)].astype(_F32)
        xb = [xt[64 * n:64 * (n + 1)] for n in range(9)]
        u = [None] + [xb[j] + xb[9 - j] for j in range(1, 5)]
        v = [None] + [xb[j] - xb[9 - j] for j in range(1, 5)]
        for k in range(1, 5):
            ar = _lin([(1.0, xb[0])] + [(_C9[j][k], u[j]) for j in range(1, 5)])
            ai = _lin([(-_S9[j][k], v[j]) for j in range(1, 5)])
            a = jnp.concatenate([ar, ai], axis=0).astype(_BF16)
            o = jnp.dot(mf_ref[k - 1], a, preferred_element_type=_F32)
            y_scr[64 * (k - 1):64 * k, pl.ds(l0, 128)] = o[:64]
            y_scr[NR + 64 * (k - 1):NR + 64 * k, pl.ds(l0, 128)] = o[64:]
        a0 = (xb[0] + (u[1] + u[2]) + (u[3] + u[4])).astype(_BF16)
        o = jnp.dot(mf_ref[4, 0:80, 0:64], a0, preferred_element_type=_F32)
        y_scr[256:NR, pl.ds(l0, 128)] = o[:40]
        y_scr[NR + 256:2 * NR, pl.ds(l0, 128)] = o[40:]

    def wnat_chunk(r0):
        wr = wrt_ref[:, pl.ds(r0, 256)].T.astype(_F32)
        wi = wit_ref[:, pl.ds(r0, 256)].T.astype(_F32)
        z = jnp.zeros((256, 128), _F32)
        for p, w in ((0, wr), (1, wi)):
            w_scr[3 * p + 0, pl.ds(r0, 256), :] = w[:, 0:128]
            w_scr[3 * p + 1, pl.ds(r0, 256), :] = w[:, 128:256]
            w_scr[3 * p + 2, pl.ds(r0, 256), :] = z
            w_scr[3 * p + 2, pl.ds(r0, 256), 0:33] = w[:, 256:289]

    def wperm_slice(k1s, ws):
        l0 = pl.multiple_of(k1s * 128, 128)
        for p in range(2):
            for t in range(3):
                blk = w_scr[3 * p + t, pl.ds(k1s, 128, stride=16), :]
                wt_scr[ws, p, 128 * t:128 * (t + 1), :] = blk.T
            for k in range(1, 5):
                wp_scr[NR * p + 64 * (k - 1):NR * p + 64 * (k - 1) + 32, pl.ds(l0, 128)] = (
                    wt_scr[ws, p, pl.ds(k, 32, stride=9), :])
                wp_scr[NR * p + 64 * (k - 1) + 32:NR * p + 64 * k, pl.ds(l0, 128)] = (
                    wt_scr[ws, p, pl.ds(9 - k, 32, stride=9), :])
            wp_scr[NR * p + 256:NR * (p + 1), pl.ds(l0, 128)] = (
                wt_scr[ws, p, pl.ds(0, 40, stride=9), :])

    for i in range(0, 2):
        copies[i].wait()
    for cp in copies[4:]:
        cp.start()

    def proj_body1b(i, carry):
        proj(2 + i)
        for j in range(4):
            wnat_chunk(pl.multiple_of(i * 1024 + j * 256, 256))
        return carry

    jax.lax.fori_loop(0, 2, proj_body1b, 0)

    for i in range(2, 4):
        copies[i].wait()

    def proj_body2(i, carry):
        proj(4 + i)
        for j in range(4):
            dfwd_tile(pl.multiple_of(i * 512 + j * 128, 128))
        for j in range(4):
            wperm_slice(4 * i + j, j)
        return carry

    jax.lax.fori_loop(0, 4, proj_body2, 0)

    for i in range(4, 8):
        copies[i].wait()
    wo_scr[...] = wo_ref[...].T

    def bfly_group(g, sign):
        r0 = pl.multiple_of(jnp.minimum(g, NG - 1) * 8, 8)
        xs = [(y_scr[pl.ds(r0, 8), 128 * n:128 * (n + 1)],
               y_scr[pl.ds(NR + r0, 8), 128 * n:128 * (n + 1)]) for n in range(16)]
        ys = _dft16(xs, sign)
        for n in range(16):
            y2_scr[pl.ds(r0, 8), 128 * n:128 * (n + 1)] = ys[n][0]
            y2_scr[pl.ds(NR + r0, 8), 128 * n:128 * (n + 1)] = ys[n][1]

    def bfly_slots(ii, sign):
        i, r = ii
        offs = ((0, 1, 2), (3, 4, 5), (6, 7), (8, 9))[r]
        pos = (1, 10, 20)
        return [(pos[n], functools.partial(bfly_group, 10 * i + o, sign))
                for n, o in enumerate(offs)]

    def stage_bfly_fwd(ii):
        return bfly_slots(ii, -1)

    def stage_bfly_inv(ii):
        return bfly_slots(ii, 1)

    def stage_smid(ii):
        k1s = ii[0] * REP + ii[1]
        l0 = pl.multiple_of(k1s * 128, 128)
        st = {}

        def part_a():
            st["p"] = jnp.dot(y2_scr[:, pl.ds(l0, 128)], gt_ref[k1s],
                              preferred_element_type=_F32)

        def part_b():
            p = st["p"]
            xr = p[:NR, :128] - p[NR:, 128:]
            xi = p[NR:, :128] + p[:NR, 128:]
            wpr = wp_scr[0:NR, pl.ds(l0, 128)]
            wpi = wp_scr[NR:2 * NR, pl.ds(l0, 128)]
            z = jnp.concatenate([xr * wpr - xi * wpi, xr * wpi + xi * wpr], axis=0)
            st["q"] = jnp.dot(z, gi_ref[k1s], preferred_element_type=_F32)

        def part_c():
            q = st["q"]
            y_scr[0:NR, pl.ds(l0, 128)] = q[:NR, :128] + q[NR:, 128:]
            y_scr[NR:2 * NR, pl.ds(l0, 128)] = q[NR:, :128] - q[:NR, 128:]

        return [(2, part_a), (12, part_b), (22, part_c)]

    def a_copy(r0, j):
        return pltpu.make_async_copy(out_scr.at[pl.ds(r0, 128), 0:512],
                                     out_hbm.at[pl.ds(r0, 128), 0:512], a_sems.at[j])

    def stage_dinv(ii):
        j = ii[0] * REP + ii[1]
        l0 = pl.multiple_of(j * 128, 128)
        st = {}

        def part_a():
            cs = []
            for k in range(1, 5):
                zz = jnp.concatenate(
                    [y2_scr[64 * (k - 1):64 * k, pl.ds(l0, 128)],
                     y2_scr[NR + 64 * (k - 1):NR + 64 * k, pl.ds(l0, 128)]],
                    axis=0).astype(_BF16)
                cs.append(jnp.dot(mi_ref[k - 1], zz, preferred_element_type=_F32))
            zz = jnp.concatenate(
                [y2_scr[256:NR, pl.ds(l0, 128)],
                 y2_scr[NR + 256:2 * NR, pl.ds(l0, 128)]], axis=0).astype(_BF16)
            st["c0"] = jnp.dot(mi_ref[4, 0:64, 0:80], zz, preferred_element_type=_F32)
            st["cs"] = cs

        def part_b():
            c0 = st["c0"]
            cr = [None] + [c[:64] for c in st["cs"]]
            ci = [None] + [c[64:] for c in st["cs"]]
            ys = [None] * 9
            ys[0] = c0 + (cr[1] + cr[2]) + (cr[3] + cr[4])
            for n in range(1, 5):
                e = _lin([(1.0, c0)] + [(_C9[n][k], cr[k]) for k in range(1, 5)])
                o = _lin([(_S9[n][k], ci[k]) for k in range(1, 5)])
                ys[n] = e - o
                ys[9 - n] = e + o
            yt = jnp.concatenate(ys, axis=0).astype(_BF16)
            out_scr[pl.ds(l0, 128), 0:D] = yt.T

        def part_c():
            a_copy(l0, j).start()

        return [(2, part_a), (12, part_b), (2 * NC - 1, part_c)]

    a_stages = (stage_bfly_fwd, stage_smid, stage_bfly_inv, stage_dinv)

    U = NQ * H
    rows128 = jax.lax.broadcasted_iota(jnp.int32, (128, TQ), 0)
    rows24q = jax.lax.broadcasted_iota(jnp.int32, (24, TQ), 0)
    rows24c = jax.lax.broadcasted_iota(jnp.int32, (24, TC), 0)

    def div7(h):
        return (h * 37) >> 8

    def tile_of(u):
        h = jnp.minimum(u, U - 1) & (H - 1)
        return pl.multiple_of(div7(h) * 128, 128)

    def qk_w(u):
        u = jnp.minimum(u, U - 1)
        qb = u >> 5
        h = u & (H - 1)
        j = h - div7(h) * HPT
        q0 = pl.multiple_of(qb * TQ, TQ)
        qt = qt_scr[pl.ds(tile_of(u), 128), pl.ds(q0, TQ)]
        mask = (rows128 >= j * DH) & (rows128 < (j + 1) * DH)
        return jnp.where(mask, qt, jnp.zeros_like(qt))

    def qk_c(qm, t0, c, slot, m):
        kt = k_scr[c * TC:(c + 1) * TC, pl.ds(t0, 128)]
        s = jnp.dot(kt, qm, preferred_element_type=_F32)
        sbuf[slot, c * TC:(c + 1) * TC, :] = s
        mc = jnp.max(s.reshape(TC // 8, 8, TQ), axis=0)
        return mc if m is None else jnp.maximum(m, mc)

    def head_rows(h):
        st = pl.multiple_of(((h * DH) >> 3) * 8, 8)
        off = h * DH - st
        return st, off, jnp.where(off == 6, 0, off + DH)

    def pv_c(st, r1, c, slot, mrow, o):
        p = jnp.exp2(sbuf[slot, c * TC:(c + 1) * TC, :] - mrow).astype(_BF16)
        vw = vt_scr[pl.ds(st, 24), c * TC:(c + 1) * TC]
        vw = jnp.where(rows24c == r1, jnp.ones_like(vw), vw)
        oc = jnp.dot(vw, p, preferred_element_type=_F32)
        return oc if o is None else o + oc

    def finalize(up, o):
        upc = jnp.maximum(up, 0)
        st, off, r1 = head_rows(upc & (H - 1))
        q0 = pl.multiple_of((upc >> 5) * TQ, TQ)
        l = jnp.sum(jnp.where(rows24q == r1, o, 0.0), axis=0, keepdims=True)
        o = o * (1.0 / l)
        omask = (rows24q >= off) & (rows24q < off + DH) & (up >= 0)
        pltpu.store(ot_scr.at[pl.ds(st, 24), pl.ds(q0, TQ)], o, mask=omask)

    def lagging(up, par_p):
        stp, _, r1p = head_rows(jnp.maximum(up, 0) & (H - 1))
        op = oacc[...]
        mp = mbuf[par_p]
        steps = []
        for c in range(LAG):
            steps.append((stp, r1p, NC - LAG + c, par_p, mp))
        return op, steps

    def step(u, par, extras=(), no_qk=False, first=False, last=False):
        st, off, r1 = head_rows(u & (H - 1))
        t0 = tile_of(u + 1)
        op, lag_steps = lagging(u - 1, 1 - par)
        mrow = jnp.max(mpart[par], axis=0, keepdims=True)
        if not no_qk:
            qm = qm_scr[...] if first else qk_w(u + 1)
        m = None
        o = None
        for c in range(NC):
            if not no_qk:
                m = qk_c(qm, t0, c, 1 - par, m)
            if c < LAG:
                op = pv_c(*lag_steps[c], op)
                if c == LAG - 1:
                    finalize(u - 1, op)
            else:
                o = pv_c(st, r1, c - LAG, par, mrow, o)
            if c == 6 and last:
                qm_scr[...] = qk_w(u + 2)
            for pos, fn in extras:
                if pos == par * NC + c:
                    fn()
        mbuf[par] = mrow
        if not no_qk:
            mpart[1 - par] = m
        oacc[...] = o

    qm0 = qk_w(jnp.int32(0))
    qm_scr[...] = qk_w(jnp.int32(1))
    m0 = None
    for c in range(NC):
        m0 = qk_c(qm0, tile_of(jnp.int32(0)), c, 0, m0)
    mpart[0] = m0
    sbuf[1, (NC - LAG) * TC:NC * TC, :] = jnp.zeros((LAG * TC, TQ), _F32)
    mbuf[1] = jnp.zeros((1, TQ), _F32)
    oacc[...] = jnp.ones((24, TQ), _F32)

    out_copies = []

    def start_out(rows, cols, k):
        cp = pltpu.make_async_copy(out_scr.at[rows[0]:rows[1], cols[0]:cols[1]],
                                   out_hbm.at[rows[0]:rows[1], cols[0]:cols[1]],
                                   out_sems.at[k])
        cp.start()
        out_copies.append(cp)

    def out_proj_tile(q0):
        ob = ot_scr[:, q0:q0 + 128].astype(_BF16)
        bt = jnp.dot(wo_scr[...], ob, preferred_element_type=_F32).astype(_BF16)
        bt = jnp.concatenate([jnp.zeros((64, 128), _BF16), bt], axis=0)
        b = bt.T
        out_scr[q0:q0 + 128, 640:1152] = b[:, 128:640]
        out_scr[q0:q0 + 128, D:640] = b[:, 64:128]

    def out_proj(qb):
        for j in range(TQ // 128):
            out_proj_tile(qb * TQ + 128 * j)

    for qb in range(NQ):
        def heads_body(i, c2, qb=qb, rep=REP):
            for r in range(rep):
                ii = i * REP + r
                u = qb * H + 2 * ii
                extras = a_stages[qb]((i, r))
                step(u, 0, extras, first=(r == 0))
                step(u + 1, 1, extras, last=(r == rep - 1))
            return c2

        if qb < NQ - 1:
            jax.lax.fori_loop(0, H // (2 * REP), heads_body, 0)
            if qb >= 1:
                out_proj(qb - 1)
                start_out(((qb - 1) * TQ, qb * TQ), (640, 1152), qb - 1)
        else:
            jax.lax.fori_loop(0, H // (2 * REP) - 1, heads_body, 0)
            if REP > 1:
                heads_body(jnp.int32(H // (2 * REP) - 1), 0, rep=REP - 1)
            extras = a_stages[qb]((jnp.int32(H // (2 * REP) - 1), REP - 1))
            step(jnp.int32(U - 2), 0, extras, first=True)
            last_extras = [(NC + 3 + 3 * j,
                            functools.partial(out_proj_tile, (qb - 1) * TQ + 128 * j))
                           for j in range(TQ // 128)]
            step(jnp.int32(U - 1), 1, list(extras) + last_extras, no_qk=True)
            start_out((0, 2 * TQ), (512, 640), NQ)
            start_out(((qb - 1) * TQ, qb * TQ), (512, 1152), qb - 1)
    op, lag_steps = lagging(jnp.int32(U - 1), 1)
    for c in range(LAG):
        op = pv_c(*lag_steps[c], op)
    finalize(jnp.int32(U - 1), op)
    for j in range(TQ // 128):
        q0 = (NQ - 1) * TQ + 128 * j
        out_proj_tile(q0)
        start_out((q0, q0 + 128), (512, 1152), NQ + 1 + j)
    for j in range(16):
        a_copy(128 * j, j).wait()
    for cp in out_copies:
        cp.wait()


@jax.jit
def pallas_concat_heads__spectral_gfnet__mha_block__prompt_kernel(
    A_x: jax.Array,
    A_w_r: jax.Array,
    A_w_i: jax.Array,
    B_x: jax.Array,
    B_wqkv: jax.Array,
    B_wo: jax.Array,
):
    xat = A_x.reshape(S, D).T
    xbt = B_x.reshape(S, D).T
    wrt = A_w_r.T
    wit = A_w_i.T
    mf = jnp.asarray(_MF, dtype=_BF16)
    mi = jnp.asarray(_MI, dtype=_BF16)
    gt = jnp.asarray(_GT, dtype=_BF16)
    gi = jnp.asarray(_GI, dtype=_BF16)

    any_spec = pl.BlockSpec(memory_space=pl.ANY)
    out = pl.pallas_call(
        _kernel,
        out_shape=jax.ShapeDtypeStruct((S, 2 * D), _BF16),
        in_specs=[any_spec] * 10,
        out_specs=any_spec,
        scratch_shapes=[
            pltpu.VMEM((D, S), _BF16),
            pltpu.VMEM((DF, S), _BF16),
            pltpu.VMEM((DF, S), _BF16),
            pltpu.VMEM((D, S), _BF16),
            pltpu.VMEM((D, 3 * D), _BF16),
            pltpu.VMEM((D, D), _BF16),
            pltpu.VMEM((5, 128, 128), _BF16),
            pltpu.VMEM((5, 128, 128), _BF16),
            pltpu.VMEM((16, 128, 256), _BF16),
            pltpu.VMEM((16, 128, 256), _BF16),
            pltpu.VMEM((S, 2 * D), _BF16),
            pltpu.SemaphoreType.DMA((8,)),
            pltpu.SemaphoreType.DMA((NQ + 1 + TQ // 128,)),
            pltpu.SemaphoreType.DMA((16,)),
            pltpu.SemaphoreType.DMA((3,)),
            pltpu.SemaphoreType.DMA((S // RC,)),
            pltpu.VMEM((S, LW), _BF16),
            pltpu.VMEM((LW, S), _BF16),
            pltpu.VMEM((D, S), _F32),
            pltpu.VMEM((D, S), _F32),
            pltpu.VMEM((2, S, TQ), _F32),
            pltpu.VMEM((2, 1, TQ), _F32),
            pltpu.VMEM((QR, D), _BF16),
            pltpu.VMEM((QR, D), _BF16),
            pltpu.VMEM((D, D), _BF16),
            pltpu.VMEM((D, D), _BF16),
            pltpu.VMEM((2 * NR, S), _F32),
            pltpu.VMEM((2 * NR, S), _F32),
            pltpu.VMEM((6, S, 128), _F32),
            pltpu.VMEM((4, 2, 384, 128), _F32),
            pltpu.VMEM((2 * NR, S), _F32),
            pltpu.VMEM((128, TQ), _BF16),
            pltpu.VMEM((2, 8, TQ), _F32),
            pltpu.VMEM((24, TQ), _F32),
        ],
        compiler_params=pltpu.CompilerParams(vmem_limit_bytes=100 * 1024 * 1024),
    )(xat, wrt, wit, xbt, B_wqkv, B_wo, mf, mi, gt, gi)
    return out.reshape(1, S, 2 * D)
```

```python
import functools
import math

import numpy as np
import jax
import jax.numpy as jnp
import jax.experimental.pallas as pl
import jax.experimental.pallas.tpu as pltpu

S = 2048
D = 576
H = 32
DH = D // H
DF = D // 2 + 1
LW = 640
TQ = 512
TC = 128
RC = 256
NQ = S // TQ
NC = S // TC
LAG = 3
REP = 4
QR = 592
HPT = 7
NR = 296
NG = NR // 8

_F32 = jnp.float32
_BF16 = jnp.bfloat16


def _dft_tables():
    n2 = np.arange(64)
    mf = np.zeros((5, 128, 128), np.float64)
    mi = np.zeros((5, 128, 128), np.float64)
    for k1 in range(1, 5):
        for part, base in ((0, k1), (1, 9 - k1)):
            sg = 1.0 if part == 0 else -1.0
            for j in range(32):
                k = base + 9 * j
                ang = 2.0 * np.pi * ((n2 * k) % D) / D
                c, s = np.cos(ang), np.sin(ang)
                rr = 32 * part + j
                ri = 64 + 32 * part + j
                mf[k1 - 1, rr, :64] = c
                mf[k1 - 1, rr, 64:] = sg * s
                mf[k1 - 1, ri, :64] = -s
                mf[k1 - 1, ri, 64:] = sg * c
                f = 2.0 / (S * D)
                mi[k1 - 1, :64, rr] = f * c
                mi[k1 - 1, :64, ri] = -f * s
                mi[k1 - 1, 64:, rr] = f * sg * s
                mi[k1 - 1, 64:, ri] = f * sg * c
    for j in range(33):
        k = 9 * j
        ang = 2.0 * np.pi * ((n2 * k) % D) / D
        c, s = np.cos(ang), np.sin(ang)
        mf[4, j, :64] = c
        mf[4, 40 + j, :64] = -s
        f = (1.0 if j in (0, 32) else 2.0) / (S * D)
        mi[4, :64, j] = f * c
        if j not in (0, 32):
            mi[4, :64, 40 + j] = -f * s
    m2 = np.arange(128)
    gt = np.zeros((16, 128, 256), np.float64)
    gi = np.zeros((16, 128, 256), np.float64)
    for k1 in range(16):
        ang = -2.0 * np.pi * (np.outer(k1 + 16 * m2, m2) % S) / S
        gt[k1, :, :128] = np.cos(ang).T
        gt[k1, :, 128:] = np.sin(ang).T
        gi[k1, :, :128] = np.cos(ang)
        gi[k1, :, 128:] = np.sin(ang)
    return mf, mi, gt, gi


_MF, _MI, _GT, _GI = _dft_tables()
_C9 = [[math.cos(2.0 * math.pi * j * k / 9.0) for k in range(5)] for j in range(5)]
_S9 = [[math.sin(2.0 * math.pi * j * k / 9.0) for k in range(5)] for j in range(5)]


def _cmul_w16(z, e, sign):
    re, im = z
    e = e % 16
    if e == 0:
        return z
    c = math.cos(2.0 * math.pi * e / 16.0)
    s = sign * math.sin(2.0 * math.pi * e / 16.0)
    if e == 4:
        return (-im, re) if sign > 0 else (im, -re)
    if e % 4 == 2:
        r = math.sqrt(0.5)
        a = re * r
        b = im * r
        cr = 1.0 if c > 0 else -1.0
        sr = 1.0 if s > 0 else -1.0
        nre = (a if cr > 0 else -a) - (b if sr > 0 else -b)
        nim = (a if sr > 0 else -a) + (b if cr > 0 else -b)
        return nre, nim
    return re * c - im * s, re * s + im * c


def _dft4(x0, x1, x2, x3, sign):
    e = (x0[0] + x2[0], x0[1] + x2[1])
    f = (x0[0] - x2[0], x0[1] - x2[1])
    g = (x1[0] + x3[0], x1[1] + x3[1])
    h = (x1[0] - x3[0], x1[1] - x3[1])
    y0 = (e[0] + g[0], e[1] + g[1])
    y2 = (e[0] - g[0], e[1] - g[1])
    if sign > 0:
        y1 = (f[0] - h[1], f[1] + h[0])
        y3 = (f[0] + h[1], f[1] - h[0])
    else:
        y1 = (f[0] + h[1], f[1] - h[0])
        y3 = (f[0] - h[1], f[1] + h[0])
    return y0, y1, y2, y3


def _dft16(xs, sign):
    t = [_dft4(xs[b], xs[4 + b], xs[8 + b], xs[12 + b], sign) for b in range(4)]
    t = [[_cmul_w16(t[b][c], b * c, sign) for c in range(4)] for b in range(4)]
    out = [None] * 16
    for c in range(4):
        ys = _dft4(t[0][c], t[1][c], t[2][c], t[3][c], sign)
        for dd in range(4):
            out[c + 4 * dd] = ys[dd]
    return out


def _lin(terms):
    acc = None
    for cf, arr in terms:
        if abs(cf) < 1e-12:
            continue
        if abs(cf - 1.0) < 1e-12:
            acc = arr if acc is None else acc + arr
        elif abs(cf + 1.0) < 1e-12:
            acc = -arr if acc is None else acc - arr
        else:
            t = arr * cf
            acc = t if acc is None else acc + t
    return acc


def _kernel(xat_hbm, wrt_hbm, wit_hbm, xbt_hbm, wqkv_hbm, wo_hbm,
            mf_hbm, mi_hbm, gt_hbm, gi_hbm,
            out_hbm,
            xat_ref, wrt_ref, wit_ref, xbt_ref, wqkv_ref, wo_ref,
            mf_ref, mi_ref, gt_ref, gi_ref,
            out_scr, in_sems, out_sems, a_sems, w_sems, x_sems,
            k_scr, qt_scr, vt_scr, ot_scr, sbuf, mbuf,
            wk_scr, wqt_scr, wvt_scr, wo_scr,
            y_scr, y2_scr, w_scr, wt_scr, wp_scr, qm_scr, mpart, oacc):
    srcs = (wrt_hbm, wit_hbm, xat_hbm, mf_hbm, wo_hbm, gt_hbm, gi_hbm, mi_hbm)
    dsts = (wrt_ref, wit_ref, xat_ref, mf_ref, wo_ref, gt_ref, gi_ref, mi_ref)
    copies = [pltpu.make_async_copy(s, d, in_sems.at[i])
              for i, (s, d) in enumerate(zip(srcs, dsts))]
    wcols = ((0, 640), (640, 1280), (1280, 3 * D))
    wcopies = [pltpu.make_async_copy(wqkv_hbm.at[:, a:b], wqkv_ref.at[:, a:b], w_sems.at[i])
               for i, (a, b) in enumerate(wcols)]

    def x_copy(c0, i):
        return pltpu.make_async_copy(xbt_hbm.at[:, pl.ds(c0, RC)],
                                     xbt_ref.at[:, pl.ds(c0, RC)], x_sems.at[i])

    wcopies[0].start()
    x_copy(0, 0).start()
    wcopies[1].start()

    qscale = (DH ** -0.5) * math.log2(math.e)

    def proj_k(r0, xt):
        kt = jnp.dot(wk_scr[...], xt, preferred_element_type=_F32).astype(_BF16)
        kt = jnp.concatenate([kt, jnp.zeros((LW - QR, RC), _BF16)], axis=0)
        k_scr[pl.ds(r0, RC), :] = kt.T

    def proj_q(r0, xt):
        qt = jnp.dot(wqt_scr[...], xt, preferred_element_type=_F32)
        qt_scr[0:QR, pl.ds(r0, RC)] = (qt * qscale).astype(_BF16)

    def proj_v(r0, xt):
        vt = jnp.dot(wvt_scr[...], xt, preferred_element_type=_F32)
        vt_scr[:, pl.ds(r0, RC)] = vt.astype(_BF16).astype(_F32)

    def proj(i):
        r0 = i * RC if isinstance(i, int) else pl.multiple_of(i * RC, RC)
        x_copy(r0, i).wait()
        xt = xbt_ref[:, pl.ds(r0, RC)]
        proj_k(r0, xt)
        proj_q(r0, xt)
        proj_v(r0, xt)

    wcopies[0].wait()
    wcopies[2].start()
    for t in range(5):
        n = 128 if t < 4 else QR - 512
        wqt_scr[128 * t:128 * t + n, :] = wqkv_ref[:, 126 * t:126 * t + 128].T[0:n]
    wcopies[1].wait()
    x_copy(0, 0).wait()
    for i in range(1, S // RC):
        x_copy(i * RC, i).start()
    proj_q(0, xbt_ref[:, 0:RC])
    for t in range(5):
        n = 128 if t < 4 else QR - 512
        wk_scr[128 * t:128 * t + n, :] = wqkv_ref[:, D + 126 * t:D + 126 * t + 128].T[0:n]
    wcopies[2].wait()
    for cp in copies[:4]:
        cp.start()
    proj_k(0, xbt_ref[:, 0:RC])
    wvt_scr[...] = wqkv_ref[:, 2 * D:3 * D].T
    proj_v(0, xbt_ref[:, 0:RC])
    proj(1)

    def dfwd_tile(l0):
        xt = xat_ref[:, pl.ds(l0, 128)].astype(_F32)
        xb = [xt[64 * n:64 * (n + 1)] for n in range(9)]
        u = [None] + [xb[j] + xb[9 - j] for j in range(1, 5)]
        v = [None] + [xb[j] - xb[9 - j] for j in range(1, 5)]
        for k in range(1, 5):
            ar = _lin([(1.0, xb[0])] + [(_C9[j][k], u[j]) for j in range(1, 5)])
            ai = _lin([(-_S9[j][k], v[j]) for j in range(1, 5)])
            a = jnp.concatenate([ar, ai], axis=0).astype(_BF16)
            o = jnp.dot(mf_ref[k - 1], a, preferred_element_type=_F32)
            y_scr[64 * (k - 1):64 * k, pl.ds(l0, 128)] = o[:64]
            y_scr[NR + 64 * (k - 1):NR + 64 * k, pl.ds(l0, 128)] = o[64:]
        a0 = (xb[0] + (u[1] + u[2]) + (u[3] + u[4])).astype(_BF16)
        o = jnp.dot(mf_ref[4, 0:80, 0:64], a0, preferred_element_type=_F32)
        y_scr[256:NR, pl.ds(l0, 128)] = o[:40]
        y_scr[NR + 256:2 * NR, pl.ds(l0, 128)] = o[40:]

    def wnat_chunk(r0):
        wr = wrt_ref[:, pl.ds(r0, 256)].T.astype(_F32)
        wi = wit_ref[:, pl.ds(r0, 256)].T.astype(_F32)
        z = jnp.zeros((256, 128), _F32)
        for p, w in ((0, wr), (1, wi)):
            w_scr[3 * p + 0, pl.ds(r0, 256), :] = w[:, 0:128]
            w_scr[3 * p + 1, pl.ds(r0, 256), :] = w[:, 128:256]
            w_scr[3 * p + 2, pl.ds(r0, 256), :] = z
            w_scr[3 * p + 2, pl.ds(r0, 256), 0:33] = w[:, 256:289]

    def wperm_slice(k1s, ws):
        l0 = pl.multiple_of(k1s * 128, 128)
        for p in range(2):
            for t in range(3):
                blk = w_scr[3 * p + t, pl.ds(k1s, 128, stride=16), :]
                wt_scr[ws, p, 128 * t:128 * (t + 1), :] = blk.T
            for k in range(1, 5):
                wp_scr[NR * p + 64 * (k - 1):NR * p + 64 * (k - 1) + 32, pl.ds(l0, 128)] = (
                    wt_scr[ws, p, pl.ds(k, 32, stride=9), :])
                wp_scr[NR * p + 64 * (k - 1) + 32:NR * p + 64 * k, pl.ds(l0, 128)] = (
                    wt_scr[ws, p, pl.ds(9 - k, 32, stride=9), :])
            wp_scr[NR * p + 256:NR * (p + 1), pl.ds(l0, 128)] = (
                wt_scr[ws, p, pl.ds(0, 40, stride=9), :])

    for i in range(0, 2):
        copies[i].wait()
    for cp in copies[4:]:
        cp.start()

    def proj_body1b(i, carry):
        proj(2 + i)
        for j in range(4):
            wnat_chunk(pl.multiple_of(i * 1024 + j * 256, 256))
        return carry

    jax.lax.fori_loop(0, 2, proj_body1b, 0)

    for i in range(2, 4):
        copies[i].wait()

    def proj_body2(i, carry):
        proj(4 + i)
        for j in range(4):
            dfwd_tile(pl.multiple_of(i * 512 + j * 128, 128))
        for j in range(4):
            wperm_slice(4 * i + j, j)
        return carry

    jax.lax.fori_loop(0, 4, proj_body2, 0)

    for i in range(4, 8):
        copies[i].wait()
    wo_scr[...] = wo_ref[...].T

    def bfly_group(g, sign):
        r0 = pl.multiple_of(jnp.minimum(g, NG - 1) * 8, 8)
        xs = [(y_scr[pl.ds(r0, 8), 128 * n:128 * (n + 1)],
               y_scr[pl.ds(NR + r0, 8), 128 * n:128 * (n + 1)]) for n in range(16)]
        ys = _dft16(xs, sign)
        for n in range(16):
            y2_scr[pl.ds(r0, 8), 128 * n:128 * (n + 1)] = ys[n][0]
            y2_scr[pl.ds(NR + r0, 8), 128 * n:128 * (n + 1)] = ys[n][1]

    def bfly_slots(ii, sign):
        i, r = ii
        offs = ((0, 1, 2), (3, 4, 5), (6, 7), (8, 9))[r]
        pos = (1, 10, 20)
        return [(pos[n], functools.partial(bfly_group, 10 * i + o, sign))
                for n, o in enumerate(offs)]

    def stage_bfly_fwd(ii):
        return bfly_slots(ii, -1)

    def stage_bfly_inv(ii):
        return bfly_slots(ii, 1)

    def stage_smid(ii):
        k1s = ii[0] * REP + ii[1]
        l0 = pl.multiple_of(k1s * 128, 128)
        st = {}

        def part_a():
            st["p"] = jnp.dot(y2_scr[:, pl.ds(l0, 128)], gt_ref[k1s],
                              preferred_element_type=_F32)

        def part_b():
            p = st["p"]
            xr = p[:NR, :128] - p[NR:, 128:]
            xi = p[NR:, :128] + p[:NR, 128:]
            wpr = wp_scr[0:NR, pl.ds(l0, 128)]
            wpi = wp_scr[NR:2 * NR, pl.ds(l0, 128)]
            z = jnp.concatenate([xr * wpr - xi * wpi, xr * wpi + xi * wpr], axis=0)
            st["q"] = jnp.dot(z, gi_ref[k1s], preferred_element_type=_F32)

        def part_c():
            q = st["q"]
            y_scr[0:NR, pl.ds(l0, 128)] = q[:NR, :128] + q[NR:, 128:]
            y_scr[NR:2 * NR, pl.ds(l0, 128)] = q[NR:, :128] - q[:NR, 128:]

        return [(2, part_a), (12, part_b), (22, part_c)]

    def a_copy(r0, j):
        return pltpu.make_async_copy(out_scr.at[pl.ds(r0, 128), 0:512],
                                     out_hbm.at[pl.ds(r0, 128), 0:512], a_sems.at[j])

    def stage_dinv(ii):
        j = ii[0] * REP + ii[1]
        l0 = pl.multiple_of(j * 128, 128)
        st = {}

        def part_a():
            cs = []
            for k in range(1, 5):
                zz = jnp.concatenate(
                    [y2_scr[64 * (k - 1):64 * k, pl.ds(l0, 128)],
                     y2_scr[NR + 64 * (k - 1):NR + 64 * k, pl.ds(l0, 128)]],
                    axis=0).astype(_BF16)
                cs.append(jnp.dot(mi_ref[k - 1], zz, preferred_element_type=_F32))
            zz = jnp.concatenate(
                [y2_scr[256:NR, pl.ds(l0, 128)],
                 y2_scr[NR + 256:2 * NR, pl.ds(l0, 128)]], axis=0).astype(_BF16)
            st["c0"] = jnp.dot(mi_ref[4, 0:64, 0:80], zz, preferred_element_type=_F32)
            st["cs"] = cs

        def part_b():
            c0 = st["c0"]
            cr = [None] + [c[:64] for c in st["cs"]]
            ci = [None] + [c[64:] for c in st["cs"]]
            ys = [None] * 9
            ys[0] = c0 + (cr[1] + cr[2]) + (cr[3] + cr[4])
            for n in range(1, 5):
                e = _lin([(1.0, c0)] + [(_C9[n][k], cr[k]) for k in range(1, 5)])
                o = _lin([(_S9[n][k], ci[k]) for k in range(1, 5)])
                ys[n] = e - o
                ys[9 - n] = e + o
            yt = jnp.concatenate(ys, axis=0).astype(_BF16)
            out_scr[pl.ds(l0, 128), 0:D] = yt.T

        def part_c():
            a_copy(l0, j).start()

        return [(2, part_a), (12, part_b), (2 * NC - 1, part_c)]

    a_stages = (stage_bfly_fwd, stage_smid, stage_bfly_inv, stage_dinv)

    U = NQ * H
    rows128 = jax.lax.broadcasted_iota(jnp.int32, (128, TQ), 0)
    rows24q = jax.lax.broadcasted_iota(jnp.int32, (24, TQ), 0)
    rows24c = jax.lax.broadcasted_iota(jnp.int32, (24, TC), 0)

    def div7(h):
        return (h * 37) >> 8

    def tile_of(u):
        h = jnp.minimum(u, U - 1) & (H - 1)
        return pl.multiple_of(div7(h) * 128, 128)

    def qk_w(u):
        u = jnp.minimum(u, U - 1)
        qb = u >> 5
        h = u & (H - 1)
        j = h - div7(h) * HPT
        q0 = pl.multiple_of(qb * TQ, TQ)
        qt = qt_scr[pl.ds(tile_of(u), 128), pl.ds(q0, TQ)]
        mask = (rows128 >= j * DH) & (rows128 < (j + 1) * DH)
        return jnp.where(mask, qt, jnp.zeros_like(qt))

    def qk_c(qm, t0, c, slot, m):
        kt = k_scr[c * TC:(c + 1) * TC, pl.ds(t0, 128)]
        s = jnp.dot(kt, qm, preferred_element_type=_F32)
        sbuf[slot, c * TC:(c + 1) * TC, :] = s
        mc = jnp.max(s.reshape(TC // 8, 8, TQ), axis=0)
        return mc if m is None else jnp.maximum(m, mc)

    def head_rows(h):
        st = pl.multiple_of(((h * DH) >> 3) * 8, 8)
        off = h * DH - st
        return st, off, jnp.where(off == 6, 0, 23)

    def pv_c(st, r1, c, slot, mrow, o):
        p = jnp.exp2(sbuf[slot, c * TC:(c + 1) * TC, :] - mrow).astype(_BF16)
        vw = vt_scr[pl.ds(st, 24), c * TC:(c + 1) * TC]
        vw = jnp.where(rows24c == r1, jnp.ones_like(vw), vw)
        oc = jnp.dot(vw, p, preferred_element_type=_F32)
        return oc if o is None else o + oc

    def finalize(up, o):
        upc = jnp.maximum(up, 0)
        st, off, r1 = head_rows(upc & (H - 1))
        q0 = pl.multiple_of((upc >> 5) * TQ, TQ)
        l = jnp.where(r1 == 0, o[0:1, :], o[23:24, :])
        r = pl.reciprocal(l, approx=True)
        r = r * (2.0 - l * r)
        o = o * r
        omask = (rows24q >= off) & (rows24q < off + DH) & (up >= 0)
        pltpu.store(ot_scr.at[pl.ds(st, 24), pl.ds(q0, TQ)], o, mask=omask)

    def lagging(up, par_p):
        stp, _, r1p = head_rows(jnp.maximum(up, 0) & (H - 1))
        op = oacc[...]
        mp = mbuf[par_p]
        steps = []
        for c in range(LAG):
            steps.append((stp, r1p, NC - LAG + c, par_p, mp))
        return op, steps

    def step(u, par, extras=(), no_qk=False, first=False, last=False):
        st, off, r1 = head_rows(u & (H - 1))
        t0 = tile_of(u + 1)
        op, lag_steps = lagging(u - 1, 1 - par)
        mrow = jnp.max(mpart[par], axis=0, keepdims=True)
        if not no_qk:
            qm = qm_scr[...] if first else qk_w(u + 1)
        m = None
        o = None
        for c in range(NC):
            if not no_qk:
                m = qk_c(qm, t0, c, 1 - par, m)
            if c < LAG:
                op = pv_c(*lag_steps[c], op)
                if c == LAG - 1:
                    finalize(u - 1, op)
            else:
                o = pv_c(st, r1, c - LAG, par, mrow, o)
            if c == 6 and last:
                qm_scr[...] = qk_w(u + 2)
            for pos, fn in extras:
                if pos == par * NC + c:
                    fn()
        mbuf[par] = mrow
        if not no_qk:
            mpart[1 - par] = m
        oacc[...] = o

    qm0 = qk_w(jnp.int32(0))
    qm_scr[...] = qk_w(jnp.int32(1))
    m0 = None
    for c in range(NC):
        m0 = qk_c(qm0, tile_of(jnp.int32(0)), c, 0, m0)
    mpart[0] = m0
    sbuf[1, (NC - LAG) * TC:NC * TC, :] = jnp.zeros((LAG * TC, TQ), _F32)
    mbuf[1] = jnp.zeros((1, TQ), _F32)
    oacc[...] = jnp.ones((24, TQ), _F32)

    out_copies = []

    def start_out(rows, cols, k):
        cp = pltpu.make_async_copy(out_scr.at[rows[0]:rows[1], cols[0]:cols[1]],
                                   out_hbm.at[rows[0]:rows[1], cols[0]:cols[1]],
                                   out_sems.at[k])
        cp.start()
        out_copies.append(cp)

    def out_proj_tile(q0):
        ob = ot_scr[:, q0:q0 + 128].astype(_BF16)
        bt = jnp.dot(wo_scr[...], ob, preferred_element_type=_F32).astype(_BF16)
        bt = jnp.concatenate([jnp.zeros((64, 128), _BF16), bt], axis=0)
        b = bt.T
        out_scr[q0:q0 + 128, 640:1152] = b[:, 128:640]
        out_scr[q0:q0 + 128, D:640] = b[:, 64:128]

    def out_proj(qb):
        for j in range(TQ // 128):
            out_proj_tile(qb * TQ + 128 * j)

    for qb in range(NQ):
        def heads_body(i, c2, qb=qb, rep=REP):
            for r in range(rep):
                ii = i * REP + r
                u = qb * H + 2 * ii
                extras = a_stages[qb]((i, r))
                step(u, 0, extras, first=(r == 0))
                step(u + 1, 1, extras, last=(r == rep - 1))
            return c2

        if qb < NQ - 1:
            jax.lax.fori_loop(0, H // (2 * REP), heads_body, 0)
            if qb >= 1:
                out_proj(qb - 1)
                start_out(((qb - 1) * TQ, qb * TQ), (640, 1152), qb - 1)
        else:
            jax.lax.fori_loop(0, H // (2 * REP) - 1, heads_body, 0)
            if REP > 1:
                heads_body(jnp.int32(H // (2 * REP) - 1), 0, rep=REP - 1)
            extras = a_stages[qb]((jnp.int32(H // (2 * REP) - 1), REP - 1))
            step(jnp.int32(U - 2), 0, extras, first=True)
            last_extras = [(NC + 3 + 3 * j,
                            functools.partial(out_proj_tile, (qb - 1) * TQ + 128 * j))
                           for j in range(TQ // 128)]
            step(jnp.int32(U - 1), 1, list(extras) + last_extras, no_qk=True)
            start_out((0, 2 * TQ), (512, 640), NQ)
            start_out(((qb - 1) * TQ, qb * TQ), (512, 1152), qb - 1)
    op, lag_steps = lagging(jnp.int32(U - 1), 1)
    for c in range(LAG):
        op = pv_c(*lag_steps[c], op)
    finalize(jnp.int32(U - 1), op)
    for j in range(TQ // 128):
        q0 = (NQ - 1) * TQ + 128 * j
        out_proj_tile(q0)
        start_out((q0, q0 + 128), (512, 1152), NQ + 1 + j)
    for j in range(16):
        a_copy(128 * j, j).wait()
    for cp in out_copies:
        cp.wait()


@jax.jit
def pallas_concat_heads__spectral_gfnet__mha_block__prompt_kernel(
    A_x: jax.Array,
    A_w_r: jax.Array,
    A_w_i: jax.Array,
    B_x: jax.Array,
    B_wqkv: jax.Array,
    B_wo: jax.Array,
):
    xat = A_x.reshape(S, D).T
    xbt = B_x.reshape(S, D).T
    wrt = A_w_r.T
    wit = A_w_i.T
    mf = jnp.asarray(_MF, dtype=_BF16)
    mi = jnp.asarray(_MI, dtype=_BF16)
    gt = jnp.asarray(_GT, dtype=_BF16)
    gi = jnp.asarray(_GI, dtype=_BF16)

    any_spec = pl.BlockSpec(memory_space=pl.ANY)
    out = pl.pallas_call(
        _kernel,
        out_shape=jax.ShapeDtypeStruct((S, 2 * D), _BF16),
        in_specs=[any_spec] * 10,
        out_specs=any_spec,
        scratch_shapes=[
            pltpu.VMEM((D, S), _BF16),
            pltpu.VMEM((DF, S), _BF16),
            pltpu.VMEM((DF, S), _BF16),
            pltpu.VMEM((D, S), _BF16),
            pltpu.VMEM((D, 3 * D), _BF16),
            pltpu.VMEM((D, D), _BF16),
            pltpu.VMEM((5, 128, 128), _BF16),
            pltpu.VMEM((5, 128, 128), _BF16),
            pltpu.VMEM((16, 128, 256), _BF16),
            pltpu.VMEM((16, 128, 256), _BF16),
            pltpu.VMEM((S, 2 * D), _BF16),
            pltpu.SemaphoreType.DMA((8,)),
            pltpu.SemaphoreType.DMA((NQ + 1 + TQ // 128,)),
            pltpu.SemaphoreType.DMA((16,)),
            pltpu.SemaphoreType.DMA((3,)),
            pltpu.SemaphoreType.DMA((S // RC,)),
            pltpu.VMEM((S, LW), _BF16),
            pltpu.VMEM((LW, S), _BF16),
            pltpu.VMEM((D, S), _F32),
            pltpu.VMEM((D, S), _F32),
            pltpu.VMEM((2, S, TQ), _F32),
            pltpu.VMEM((2, 1, TQ), _F32),
            pltpu.VMEM((QR, D), _BF16),
            pltpu.VMEM((QR, D), _BF16),
            pltpu.VMEM((D, D), _BF16),
            pltpu.VMEM((D, D), _BF16),
            pltpu.VMEM((2 * NR, S), _F32),
            pltpu.VMEM((2 * NR, S), _F32),
            pltpu.VMEM((6, S + 16, 128), _F32),
            pltpu.VMEM((4, 2, 384, 128), _F32),
            pltpu.VMEM((2 * NR, S), _F32),
            pltpu.VMEM((128, TQ), _BF16),
            pltpu.VMEM((2, 8, TQ), _F32),
            pltpu.VMEM((24, TQ), _F32),
        ],
        compiler_params=pltpu.CompilerParams(vmem_limit_bytes=100 * 1024 * 1024),
    )(xat, wrt, wit, xbt, B_wqkv, B_wo, mf, mi, gt, gi)
    return out.reshape(1, S, 2 * D)
```
